```python
import jax
import jax.numpy as jnp

def _softmax(x, axis=-1):
    return jax.nn.softmax(x, axis=axis)
def _gelu(x):
    return jax.nn.gelu(x, approximate=True)
def _silu(x):
    return jax.nn.silu(x)
def _sigmoid(x):
    return jax.nn.sigmoid(x)
def _layernorm(x, axis=-1, eps=1e-5):
    m = jnp.mean(x, axis=axis, keepdims=True)
    v = jnp.var(x, axis=axis, keepdims=True)
    return (x - m) / jnp.sqrt(v + eps)
def _scatter_add(tgt, idx, src, axis=0):
    return tgt.at[idx].add(src)
def _segment_sum(src, seg, n):
    return jax.ops.segment_sum(src, seg, n)
class _Rng:
    def __init__(self, key):
        self._k = key
    def _next(self):
        self._k, sub = jax.random.split(self._k)
        return sub
    def normal(self, shape):
        return jax.random.normal(self._next(), shape, dtype=jnp.bfloat16)
    def randint(self, lo, hi, shape):
        return jax.random.randint(self._next(), shape, lo, hi, dtype=jnp.int32)
    def uniform(self, shape, lo=0.0, hi=1.0):
        return jax.random.uniform(self._next(), shape, jnp.bfloat16, lo, hi)
    def permutation(self, n):
        return jax.random.permutation(self._next(), n)


kernel_name = 'sequential_preLN__sliding_block__glu_gated_glu__prompt'

def _fwd_setup_inputs():
    _rng = _Rng(jax.random.key(int.from_bytes(__import__("os").urandom(4), "little")))
    _w = (lambda a: (lambda t: t.astype(jnp.bfloat16) if jnp.issubdtype(t.dtype, jnp.floating) else t)(jnp.asarray(a)))
    def _A_setup():
        B, S, D = 1, 2048, 512
        return {
            "x": _w((lambda *s: _rng.normal(s) * 0.05)(B, S, D)),
            "wqkv": _w((lambda *s: _rng.normal(s) * 0.05)(D, 3 * D)),
            "wo": _w((lambda *s: _rng.normal(s) * 0.05)(D, D)),
        }
    _A_in = _A_setup()

    def _B_setup():
        B, S, D, F = 1, 2048, 512, 1376
        return {
            "x": _w((lambda *s: _rng.normal(s) * 0.05)(B, S, D)),
            "w_gate": _w((lambda *s: _rng.normal(s) * 0.05)(D, F)),
            "w_up": _w((lambda *s: _rng.normal(s) * 0.05)(D, F)),
            "w_down": _w((lambda *s: _rng.normal(s) * 0.05)(F, D)),
        }
    _B_in = _B_setup()

    return {
        "A_x": _A_in["x"],
        "A_wqkv": _A_in["wqkv"],
        "A_wo": _A_in["wo"],
        "B_x": _B_in["x"],
        "B_w_gate": _B_in["w_gate"],
        "B_w_up": _B_in["w_up"],
        "B_w_down": _B_in["w_down"],
    }

def _fwd_reference(A_x, A_wqkv, A_wo, B_x, B_w_gate, B_w_up, B_w_down):
    def _A_ref(x, wqkv, wo):
        B, S, D = x.shape
        H = 32; Dh = D // H; W = 256
        qkv = (lambda x, *d: x.transpose(*d))((x @ wqkv).reshape(B, S, 3, H, Dh), 2, 0, 3, 1, 4)
        q, k, v = qkv[0], qkv[1], qkv[2]
        scores = jnp.einsum("bhqd,bhkd->bhqk", q, k) * (Dh ** -0.5)
        idx = jnp.arange(S)
        mask = (idx[:, None] - idx[None, :] >= 0) & (idx[:, None] - idx[None, :] < W)
        scores = jnp.where(mask[None, None], scores, -1e9)
        p = _softmax(scores, axis=-1)
        o = jnp.einsum("bhqk,bhkd->bhqd", p, v)
        return (lambda x, *d: x.transpose(*d))(o, 0, 2, 1, 3).reshape(B, S, D) @ wo

    def _B_ref(x, w_gate, w_up, w_down):
        g = jnp.einsum("bsd,df->bsf", x, w_gate)
        u = jnp.einsum("bsd,df->bsf", x, w_up)
        h = _sigmoid(g) * u
        return jnp.einsum("bsf,fd->bsd", h, w_down)

    x = A_x
    h = x + _A_ref(_layernorm(x, axis=-1), A_wqkv, A_wo)
    h2 = h + _B_ref(_layernorm(h, axis=-1), B_w_gate, B_w_up, B_w_down)
    return h2


def setup_inputs():
    _inp = _fwd_setup_inputs()
    _gk = jax.random.fold_in(jax.random.key(int.from_bytes(__import__("os").urandom(4), "little")), 2**31 - 1)
    _shapes = [[1, 2048, 512]]
    _dtypes = ['bfloat16']
    _gks = jax.random.split(_gk, len(_shapes))
    _gs = [jax.random.normal(k, s, dtype=jnp.dtype(d)) * 0.05 for k, s, d in zip(_gks, _shapes, _dtypes)]
    _inp["grad_out"] = _gs[0]
    return _inp

def reference(A_x, A_wqkv, A_wo, B_w_gate, B_w_up, B_w_down, B_x, grad_out):
    _const = dict(B_x=B_x)
    def _f(*_d):
        return _fwd_reference(**{'A_x': _d[0], 'A_wqkv': _d[1], 'A_wo': _d[2], 'B_w_gate': _d[3], 'B_w_up': _d[4], 'B_w_down': _d[5], **_const})
    _out, _vjp = jax.vjp(_f, A_x, A_wqkv, A_wo, B_w_gate, B_w_up, B_w_down)
    _grads = _vjp(grad_out)
    _out0 = jnp.asarray(_out)
    return (_out0, *[jnp.asarray(_g) for _g in _grads])
```

```python
import jax
import jax.numpy as jnp
from jax import lax
import jax.experimental.pallas as pl
import jax.experimental.pallas.tpu as pltpu

S, D, F = 2048, 512, 1376
H, DH, W = 32, 16, 256
QB = 128
KW = QB + W
NG = D // 128
HG = 128 // DH
SB = 256
NSB = S // SB
RC = 512
EPS = 1e-5
NEG = -1e9
F32 = jnp.float32
BF16 = jnp.bfloat16


def _nn(a, b):
    return jnp.dot(a, b, preferred_element_type=F32)


def _nt(a, b):
    return lax.dot_general(a, b, (((1,), (1,)), ((), ())), preferred_element_type=F32)


def _tn(a, b):
    return lax.dot_general(a, b, (((0,), (0,)), ((), ())), preferred_element_type=F32)


def _ln(x):
    m = jnp.mean(x, axis=-1, keepdims=True)
    xc = x - m
    v = jnp.mean(xc * xc, axis=-1, keepdims=True)
    r = lax.rsqrt(v + EPS)
    return xc * r, r


def _ln_bwd(dy, y, r):
    a = jnp.mean(dy, axis=-1, keepdims=True)
    b = jnp.mean(dy * y, axis=-1, keepdims=True)
    return r * (dy - a - y * b)


def _kernel(x_ref, wqkv_ref, wo_ref, wg_ref, wu_ref, wd_ref, go_ref,
            out_ref, dx_ref, dwqkv_ref, dwo_ref, dwg_ref, dwu_ref, dwd_ref,
            ln1_s, q_s, k_s, v_s, o_s, p_s, h_s, do_s, ln2_s, hh_s, dg_s, du_s,
            dh_s, dq_s, dk_s, dv_s, dqkv_s):
    k_s[0:W, :] = jnp.zeros((W, D), BF16)
    v_s[0:W, :] = jnp.zeros((W, D), BF16)
    dk_s[...] = jnp.zeros(dk_s.shape, F32)
    dv_s[...] = jnp.zeros(dv_s.shape, F32)

    def p1(c, carry):
        r0 = pl.multiple_of(c * RC, RC)
        x = x_ref[pl.ds(r0, RC), :].astype(F32)
        y, _ = _ln(x)
        yb = y.astype(BF16)
        ln1_s[pl.ds(r0, RC), :] = yb
        qkv = _nn(yb, wqkv_ref[...])
        q_s[pl.ds(r0, RC), :] = (qkv[:, 0:D] * (DH ** -0.5)).astype(BF16)
        k_s[pl.ds(r0 + W, RC), :] = qkv[:, D:2 * D].astype(BF16)
        v_s[pl.ds(r0 + W, RC), :] = qkv[:, 2 * D:3 * D].astype(BF16)
        return carry

    lax.fori_loop(0, S // RC, p1, 0)

    head_of_lane = lax.broadcasted_iota(jnp.int32, (HG, 1, 128), 2) // DH
    head_id = lax.broadcasted_iota(jnp.int32, (HG, 1, 128), 0)
    hmask = head_of_lane == head_id

    def stack_heads(t):
        return jnp.where(hmask, t[None], jnp.zeros_like(t)[None]).reshape(HG * QB, 128)

    def unstack_heads(t):
        return jnp.sum(jnp.where(hmask, t.reshape(HG, QB, 128), 0.0), axis=0)

    def win_mask(qi):
        r = lax.broadcasted_iota(jnp.int32, (QB, KW), 0)
        c = lax.broadcasted_iota(jnp.int32, (QB, KW), 1)
        return (c > r) & (c <= r + W) & (c >= (2 - qi) * QB)

    def p2(sb, carry):
        r0 = pl.multiple_of(sb * SB, SB)

        def attn_fwd(t, c2):
            qb = t // NG
            g = t % NG
            qi = sb * (SB // QB) + qb
            q0 = pl.multiple_of(qi * QB, QB)
            l0 = pl.multiple_of(g * 128, 128)
            qg = q_s[pl.ds(q0, QB), pl.ds(l0, 128)]
            kg = k_s[pl.ds(q0, KW), pl.ds(l0, 128)]
            vg = v_s[pl.ds(q0, KW), pl.ds(l0, 128)]
            s = _nt(stack_heads(qg), kg).reshape(HG, QB, KW)
            s = jnp.where(win_mask(qi)[None], s, NEG)
            m = jnp.max(s, axis=-1, keepdims=True)
            p = jnp.exp(s - m)
            l = jnp.sum(p, axis=-1, keepdims=True)
            pn = (p / l).astype(BF16).reshape(HG * QB, KW)
            p_s[t] = pn
            o = unstack_heads(_nn(pn, vg))
            o_s[pl.ds(q0, QB), pl.ds(l0, 128)] = o.astype(BF16)
            return c2

        lax.fori_loop(0, (SB // QB) * NG, attn_fwd, 0)

        rows = pl.ds(r0, SB)
        x = x_ref[rows, :].astype(F32)
        h = x + _nn(o_s[rows, :], wo_ref[...])
        y2, r2 = _ln(h)
        y2b = y2.astype(BF16)
        ln2_s[rows, :] = y2b
        gt = _nn(y2b, wg_ref[...])
        u = _nn(y2b, wu_ref[...])
        sg = jax.nn.sigmoid(gt)
        hh = (sg * u).astype(BF16)
        hh_s[rows, :] = hh
        out_ref[rows, :] = (h + _nn(hh, wd_ref[...])).astype(BF16)

        go = go_ref[rows, :]
        dhh = _nt(go, wd_ref[...])
        du = dhh * sg
        dg = du * u * (1.0 - sg)
        dub = du.astype(BF16)
        dgb = dg.astype(BF16)
        du_s[rows, :] = dub
        dg_s[rows, :] = dgb
        dy2 = _nt(dgb, wg_ref[...]) + _nt(dub, wu_ref[...])
        dh = go.astype(F32) + _ln_bwd(dy2, y2, r2)
        dh_s[rows, :] = dh
        do_s[...] = _nt(dh.astype(BF16), wo_ref[...]).astype(BF16)

        def attn_bwd(t, c2):
            qb = t // NG
            g = t % NG
            qi = sb * (SB // QB) + qb
            q0 = pl.multiple_of(qi * QB, QB)
            l0 = pl.multiple_of(g * 128, 128)
            qm = stack_heads(q_s[pl.ds(q0, QB), pl.ds(l0, 128)])
            kg = k_s[pl.ds(q0, KW), pl.ds(l0, 128)]
            vg = v_s[pl.ds(q0, KW), pl.ds(l0, 128)]
            dom = stack_heads(do_s[pl.ds(pl.multiple_of(qb * QB, QB), QB), pl.ds(l0, 128)])
            pn = p_s[t]
            pf = pn.astype(F32)
            dp = _nt(dom, vg)
            delta = jnp.sum(dp * pf, axis=-1, keepdims=True)
            ds = (pf * (dp - delta)).astype(BF16)
            dq = unstack_heads(_nn(ds, kg)) * (DH ** -0.5)
            dq_s[pl.ds(q0, QB), pl.ds(l0, 128)] = dq.astype(BF16)
            dk_s[pl.ds(q0, KW), pl.ds(l0, 128)] += _tn(ds, qm)
            dv_s[pl.ds(q0, KW), pl.ds(l0, 128)] += _tn(pn, dom)
            return c2

        lax.fori_loop(0, (SB // QB) * NG, attn_bwd, 0)
        return carry

    lax.fori_loop(0, NSB, p2, 0)

    def p3(c, carry):
        r0 = pl.multiple_of(c * RC, RC)
        rows = pl.ds(r0, RC)
        dqkv_s[rows, 0:D] = dq_s[rows, :]
        dqkv_s[rows, D:2 * D] = dk_s[pl.ds(r0 + W, RC), :].astype(BF16)
        dqkv_s[rows, 2 * D:3 * D] = dv_s[pl.ds(r0 + W, RC), :].astype(BF16)
        dy1 = _nt(dqkv_s[rows, :], wqkv_ref[...])
        x = x_ref[rows, :].astype(F32)
        y1, r1 = _ln(x)
        dx_ref[rows, :] = (dh_s[rows, :] + _ln_bwd(dy1, y1, r1)).astype(BF16)
        return carry

    lax.fori_loop(0, S // RC, p3, 0)

    dwqkv_ref[...] = _tn(ln1_s[...], dqkv_s[...]).astype(BF16)
    dwo_ref[...] = _tn(o_s[...], dh_s[...].astype(BF16)).astype(BF16)
    dwg_ref[...] = _tn(ln2_s[...], dg_s[...]).astype(BF16)
    dwu_ref[...] = _tn(ln2_s[...], du_s[...]).astype(BF16)
    dwd_ref[...] = _tn(hh_s[...], go_ref[...]).astype(BF16)


@jax.jit
def pallas_sequential_preLN__sliding_block__glu_gated_glu__prompt_kernel(
    A_x: jax.Array,
    A_wqkv: jax.Array,
    A_wo: jax.Array,
    B_x: jax.Array,
    B_w_gate: jax.Array,
    B_w_up: jax.Array,
    B_w_down: jax.Array,
    grad_out: jax.Array,
):
    del B_x
    x = A_x.reshape(S, D)
    go = grad_out.reshape(S, D)
    sds = jax.ShapeDtypeStruct
    out_shape = (
        sds((S, D), BF16), sds((S, D), BF16),
        sds((D, 3 * D), BF16), sds((D, D), BF16),
        sds((D, F), BF16), sds((D, F), BF16), sds((F, D), BF16),
    )
    scratch = [
        pltpu.VMEM((S, D), BF16),
        pltpu.VMEM((S, D), BF16),
        pltpu.VMEM((S + W, D), BF16),
        pltpu.VMEM((S + W, D), BF16),
        pltpu.VMEM((S, D), BF16),
        pltpu.VMEM(((SB // QB) * NG, HG * QB, KW), BF16),
        pltpu.VMEM((SB, D), F32),
        pltpu.VMEM((SB, D), BF16),
        pltpu.VMEM((S, D), BF16),
        pltpu.VMEM((S, F), BF16),
        pltpu.VMEM((S, F), BF16),
        pltpu.VMEM((S, F), BF16),
        pltpu.VMEM((S, D), F32),
        pltpu.VMEM((S, D), BF16),
        pltpu.VMEM((S + W, D), F32),
        pltpu.VMEM((S + W, D), F32),
        pltpu.VMEM((S, 3 * D), BF16),
    ]
    outs = pl.pallas_call(
        _kernel,
        out_shape=out_shape,
        scratch_shapes=scratch,
        compiler_params=pltpu.CompilerParams(vmem_limit_bytes=120 * 1024 * 1024),
    )(x, A_wqkv, A_wo, B_w_gate, B_w_up, B_w_down, go)
    out, dx = outs[0].reshape(1, S, D), outs[1].reshape(1, S, D)
    return (out, dx) + tuple(outs[2:])
```

```python
import jax
import jax.numpy as jnp
from jax import lax
import jax.experimental.pallas as pl
import jax.experimental.pallas.tpu as pltpu

S, D, F = 2048, 512, 1376
H, DH, W = 32, 16, 256
QB = 128
KW = QB + W
NG = D // 128
HG = 128 // DH
SB = 256
NSB = S // SB
RC = 512
EPS = 1e-5
NEG = -1e9
F32 = jnp.float32
BF16 = jnp.bfloat16


def _nn(a, b):
    return jnp.dot(a, b, preferred_element_type=F32)


def _nt(a, b):
    return lax.dot_general(a, b, (((1,), (1,)), ((), ())), preferred_element_type=F32)


def _tn(a, b):
    return lax.dot_general(a, b, (((0,), (0,)), ((), ())), preferred_element_type=F32)


def _ln(x):
    m = jnp.mean(x, axis=-1, keepdims=True)
    xc = x - m
    v = jnp.mean(xc * xc, axis=-1, keepdims=True)
    r = lax.rsqrt(v + EPS)
    return xc * r, r


def _ln_bwd(dy, y, r):
    a = jnp.mean(dy, axis=-1, keepdims=True)
    b = jnp.mean(dy * y, axis=-1, keepdims=True)
    return r * (dy - a - y * b)


def _kernel(x_ref, wqkv_ref, wo_ref, wg_ref, wu_ref, wd_ref, go_ref,
            out_ref, dx_ref, dwqkv_ref, dwo_ref, dwg_ref, dwu_ref, dwd_ref,
            ln1_s, q_s, qT_s, k_s, kT_s, v_s, vT_s, o_s, p_s, do_s, doT_s, ln2_s, hh_s,
            dg_s, du_s, dh_s, dq_s, dkT_s, dvT_s, dqkv_s):
    k_s[0:W, :] = jnp.zeros((W, D), BF16)
    v_s[0:W, :] = jnp.zeros((W, D), BF16)
    kT_s[:, 0:W] = jnp.zeros((D, W), BF16)
    vT_s[:, 0:W] = jnp.zeros((D, W), BF16)
    dkT_s[...] = jnp.zeros(dkT_s.shape, F32)
    dvT_s[...] = jnp.zeros(dvT_s.shape, F32)

    def p1(c, carry):
        r0 = pl.multiple_of(c * RC, RC)
        x = x_ref[pl.ds(r0, RC), :].astype(F32)
        y, _ = _ln(x)
        yb = y.astype(BF16)
        ln1_s[pl.ds(r0, RC), :] = yb
        qkv = _nn(yb, wqkv_ref[...])
        q = (qkv[:, 0:D] * (DH ** -0.5)).astype(BF16)
        k = qkv[:, D:2 * D].astype(BF16)
        v = qkv[:, 2 * D:3 * D].astype(BF16)
        q_s[pl.ds(r0, RC), :] = q
        k_s[pl.ds(r0 + W, RC), :] = k
        v_s[pl.ds(r0 + W, RC), :] = v
        qT_s[:, pl.ds(r0, RC)] = q.T
        kT_s[:, pl.ds(r0 + W, RC)] = k.T
        vT_s[:, pl.ds(r0 + W, RC)] = v.T
        return carry

    with jax.named_scope("p1_qkv"):
        lax.fori_loop(0, S // RC, p1, 0)

    head_of_lane = lax.broadcasted_iota(jnp.int32, (QB, 128), 1) // DH

    def win_mask_t(qi):
        c = lax.broadcasted_iota(jnp.int32, (KW, QB), 0)
        r = lax.broadcasted_iota(jnp.int32, (KW, QB), 1)
        return (c > r) & (c <= r + W) & (c >= (2 - qi) * QB)

    def p2(sb, carry):
        r0 = pl.multiple_of(sb * SB, SB)

        def attn_fwd(t, c2):
            qb = t // NG
            g = t % NG
            qi = sb * (SB // QB) + qb
            q0 = pl.multiple_of(qi * QB, QB)
            l0 = pl.multiple_of(g * 128, 128)
            qg = q_s[pl.ds(q0, QB), pl.ds(l0, 128)]
            kg = k_s[pl.ds(q0, KW), pl.ds(l0, 128)]
            msk = win_mask_t(qi)
            o_parts = []
            for j in range(HG):
                qm = jnp.where(head_of_lane == j, qg, jnp.zeros_like(qg))
                s = jnp.where(msk, _nt(kg, qm), NEG)
                m = jnp.max(s, axis=0, keepdims=True)
                p = jnp.exp(s - m)
                l = jnp.sum(p, axis=0, keepdims=True)
                pn = (p * (1.0 / l)).astype(BF16)
                p_s[t, j] = pn
                vt = vT_s[pl.ds(pl.multiple_of(l0 + j * DH, DH), DH), pl.ds(q0, KW)]
                o_parts.append(_nn(vt, pn))
            ot = jnp.concatenate(o_parts, axis=0)
            o_s[pl.ds(q0, QB), pl.ds(l0, 128)] = ot.T.astype(BF16)
            return c2

        with jax.named_scope("attn_fwd"):
            lax.fori_loop(0, (SB // QB) * NG, attn_fwd, 0)

        rows = pl.ds(r0, SB)
        x = x_ref[rows, :].astype(F32)
        h = x + _nn(o_s[rows, :], wo_ref[...])
        y2, r2 = _ln(h)
        y2b = y2.astype(BF16)
        ln2_s[rows, :] = y2b
        gt = _nn(y2b, wg_ref[...])
        u = _nn(y2b, wu_ref[...])
        sg = jax.nn.sigmoid(gt)
        hh = (sg * u).astype(BF16)
        hh_s[rows, :] = hh
        out_ref[rows, :] = (h + _nn(hh, wd_ref[...])).astype(BF16)

        go = go_ref[rows, :]
        dhh = _nt(go, wd_ref[...])
        du = dhh * sg
        dg = du * u * (1.0 - sg)
        dub = du.astype(BF16)
        dgb = dg.astype(BF16)
        du_s[rows, :] = dub
        dg_s[rows, :] = dgb
        dy2 = _nt(dgb, wg_ref[...]) + _nt(dub, wu_ref[...])
        dh = go.astype(F32) + _ln_bwd(dy2, y2, r2)
        dh_s[rows, :] = dh
        do = _nt(dh.astype(BF16), wo_ref[...]).astype(BF16)
        do_s[...] = do
        doT_s[...] = do.T

        def attn_bwd(t, c2):
            qb = t // NG
            g = t % NG
            qi = sb * (SB // QB) + qb
            q0 = pl.multiple_of(qi * QB, QB)
            b0 = pl.multiple_of(qb * QB, QB)
            l0 = pl.multiple_of(g * 128, 128)
            dog = do_s[pl.ds(b0, QB), pl.ds(l0, 128)]
            vg = v_s[pl.ds(q0, KW), pl.ds(l0, 128)]
            dq_parts = []
            for j in range(HG):
                hl = pl.ds(pl.multiple_of(l0 + j * DH, DH), DH)
                dom = jnp.where(head_of_lane == j, dog, jnp.zeros_like(dog))
                pn = p_s[t, j]
                pf = pn.astype(F32)
                dp = _nt(vg, dom)
                delta = jnp.sum(pf * dp, axis=0, keepdims=True)
                ds = (pf * (dp - delta)).astype(BF16)
                dq_parts.append(_nn(kT_s[hl, pl.ds(q0, KW)], ds))
                dkT_s[hl, pl.ds(q0, KW)] += _nt(qT_s[hl, pl.ds(q0, QB)], ds)
                dvT_s[hl, pl.ds(q0, KW)] += _nt(doT_s[hl, pl.ds(b0, QB)], pn)
            dqt = jnp.concatenate(dq_parts, axis=0) * (DH ** -0.5)
            dq_s[pl.ds(q0, QB), pl.ds(l0, 128)] = dqt.T.astype(BF16)
            return c2

        with jax.named_scope("attn_bwd"):
            lax.fori_loop(0, (SB // QB) * NG, attn_bwd, 0)
        return carry

    with jax.named_scope("p2_all"):
        lax.fori_loop(0, NSB, p2, 0)

    def p3(c, carry):
        r0 = pl.multiple_of(c * RC, RC)
        rows = pl.ds(r0, RC)
        dqkv_s[rows, 0:D] = dq_s[rows, :]
        dqkv_s[rows, D:2 * D] = dkT_s[:, pl.ds(r0 + W, RC)].T.astype(BF16)
        dqkv_s[rows, 2 * D:3 * D] = dvT_s[:, pl.ds(r0 + W, RC)].T.astype(BF16)
        dy1 = _nt(dqkv_s[rows, :], wqkv_ref[...])
        x = x_ref[rows, :].astype(F32)
        y1, r1 = _ln(x)
        dx_ref[rows, :] = (dh_s[rows, :] + _ln_bwd(dy1, y1, r1)).astype(BF16)
        return carry

    with jax.named_scope("p3"):
        lax.fori_loop(0, S // RC, p3, 0)

    with jax.named_scope("p4_wgrad"):
        dwqkv_ref[...] = _tn(ln1_s[...], dqkv_s[...]).astype(BF16)
        dwo_ref[...] = _tn(o_s[...], dh_s[...].astype(BF16)).astype(BF16)
        dwg_ref[...] = _tn(ln2_s[...], dg_s[...]).astype(BF16)
        dwu_ref[...] = _tn(ln2_s[...], du_s[...]).astype(BF16)
        dwd_ref[...] = _tn(hh_s[...], go_ref[...]).astype(BF16)


@jax.jit
def pallas_sequential_preLN__sliding_block__glu_gated_glu__prompt_kernel(
    A_x: jax.Array,
    A_wqkv: jax.Array,
    A_wo: jax.Array,
    B_x: jax.Array,
    B_w_gate: jax.Array,
    B_w_up: jax.Array,
    B_w_down: jax.Array,
    grad_out: jax.Array,
):
    del B_x
    x = A_x.reshape(S, D)
    go = grad_out.reshape(S, D)
    sds = jax.ShapeDtypeStruct
    out_shape = (
        sds((S, D), BF16), sds((S, D), BF16),
        sds((D, 3 * D), BF16), sds((D, D), BF16),
        sds((D, F), BF16), sds((D, F), BF16), sds((F, D), BF16),
    )
    scratch = [
        pltpu.VMEM((S, D), BF16),
        pltpu.VMEM((S, D), BF16),
        pltpu.VMEM((D, S), BF16),
        pltpu.VMEM((S + W, D), BF16),
        pltpu.VMEM((D, S + W), BF16),
        pltpu.VMEM((S + W, D), BF16),
        pltpu.VMEM((D, S + W), BF16),
        pltpu.VMEM((S, D), BF16),
        pltpu.VMEM(((SB // QB) * NG, HG, KW, QB), BF16),
        pltpu.VMEM((SB, D), BF16),
        pltpu.VMEM((D, SB), BF16),
        pltpu.VMEM((S, D), BF16),
        pltpu.VMEM((S, F), BF16),
        pltpu.VMEM((S, F), BF16),
        pltpu.VMEM((S, F), BF16),
        pltpu.VMEM((S, D), F32),
        pltpu.VMEM((S, D), BF16),
        pltpu.VMEM((D, S + W), F32),
        pltpu.VMEM((D, S + W), F32),
        pltpu.VMEM((S, 3 * D), BF16),
    ]
    outs = pl.pallas_call(
        _kernel,
        out_shape=out_shape,
        scratch_shapes=scratch,
        compiler_params=pltpu.CompilerParams(vmem_limit_bytes=120 * 1024 * 1024),
    )(x, A_wqkv, A_wo, B_w_gate, B_w_up, B_w_down, go)
    out, dx = outs[0].reshape(1, S, D), outs[1].reshape(1, S, D)
    return (out, dx) + tuple(outs[2:])
```

```python
import jax
import jax.numpy as jnp
from jax import lax
import jax.experimental.pallas as pl
import jax.experimental.pallas.tpu as pltpu

S, D, F = 2048, 512, 1376
H, DH, W = 32, 16, 256
QB = 128
KW = QB + W
NG = D // 128
HG = 128 // DH
SB = 256
NSB = S // SB
NT = (SB // QB) * NG
RC = 512
EPS = 1e-5
NEG = -1e9
SCALE = DH ** -0.5
LOG2E = 1.4426950408889634
F32 = jnp.float32
BF16 = jnp.bfloat16


def _nn(a, b):
    return jnp.dot(a, b, preferred_element_type=F32)


def _nt(a, b):
    return lax.dot_general(a, b, (((1,), (1,)), ((), ())), preferred_element_type=F32)


def _tn(a, b):
    return lax.dot_general(a, b, (((0,), (0,)), ((), ())), preferred_element_type=F32)


def _ln(x):
    m = jnp.mean(x, axis=-1, keepdims=True)
    xc = x - m
    v = jnp.mean(xc * xc, axis=-1, keepdims=True)
    r = lax.rsqrt(v + EPS)
    return xc * r, r


def _ln_bwd(dy, y, r):
    a = jnp.mean(dy, axis=-1, keepdims=True)
    b = jnp.mean(dy * y, axis=-1, keepdims=True)
    return r * (dy - a - y * b)


def _kernel(x_ref, wqkv_ref, wo_ref, wg_ref, wu_ref, wd_ref, go_ref,
            out_ref, dx_ref, dwqkv_ref, dwo_ref, dwg_ref, dwu_ref, dwd_ref,
            ln1_s, q_s, qT_s, k_s, kT_s, v_s, vT_s, o_s, oT_s, il_s, p_s, doT_s, ln2_s, hh_s,
            dg_s, du_s, dh_s, dq_s, dkT_s, dvT_s, dqkv_s, bufA, bufB, mb_s):
    k_s[0:W, :] = jnp.zeros((W, D), BF16)
    v_s[0:W, :] = jnp.zeros((W, D), BF16)
    kT_s[:, 0:W] = jnp.zeros((D, W), BF16)
    vT_s[:, 0:W] = jnp.zeros((D, W), BF16)
    dkT_s[...] = jnp.zeros(dkT_s.shape, F32)
    dvT_s[...] = jnp.zeros(dvT_s.shape, F32)

    c_i = lax.broadcasted_iota(jnp.int32, (KW, QB), 0)
    r_i = lax.broadcasted_iota(jnp.int32, (KW, QB), 1)
    for var in range(3):
        ok = (c_i > r_i) & (c_i <= r_i + W) & (c_i >= (2 - var) * QB)
        mb_s[var] = jnp.where(ok, 0.0, NEG)

    def p1(c, carry):
        r0 = pl.multiple_of(c * RC, RC)
        x = x_ref[pl.ds(r0, RC), :].astype(F32)
        y, _ = _ln(x)
        yb = y.astype(BF16)
        ln1_s[pl.ds(r0, RC), :] = yb
        qkv = _nn(yb, wqkv_ref[...])
        q = qkv[:, 0:D]
        k = qkv[:, D:2 * D]
        v = qkv[:, 2 * D:3 * D]
        q_s[pl.ds(r0, RC), :] = (q * (SCALE * LOG2E)).astype(BF16)
        k_s[pl.ds(r0 + W, RC), :] = k.astype(BF16)
        v_s[pl.ds(r0 + W, RC), :] = v.astype(BF16)
        qT_s[:, pl.ds(r0, RC)] = (q * SCALE).T.astype(BF16)
        kT_s[:, pl.ds(r0 + W, RC)] = k.T.astype(BF16)
        vT_s[:, pl.ds(r0 + W, RC)] = v.T.astype(BF16)
        return carry

    with jax.named_scope("p1_qkv"):
        lax.fori_loop(0, S // RC, p1, 0)

    head_of_lane = lax.broadcasted_iota(jnp.int32, (QB, 128), 1) // DH
    head_of_row = lax.broadcasted_iota(jnp.int32, (128, QB), 0) // DH

    def p2(sb, carry):
        r0 = pl.multiple_of(sb * SB, SB)

        def idx(t):
            qi = sb * (SB // QB) + t // NG
            g = t % NG
            return qi, pl.multiple_of(qi * QB, QB), pl.multiple_of(g * 128, 128)

        def qk_j(t, dst, j):
            qi, q0, l0 = idx(t)
            qg = q_s[pl.ds(q0, QB), pl.ds(l0, 128)]
            kg = k_s[pl.ds(q0, KW), pl.ds(l0, 128)]
            qm = jnp.where(head_of_lane == j, qg, jnp.zeros_like(qg))
            dst[j] = _nt(kg, qm) + mb_s[jnp.minimum(qi, 2)]

        def sm_pv_j(t, src, j):
            qi, q0, l0 = idx(t)
            s = src[j]
            m = jnp.max(s, axis=0, keepdims=True)
            p = jnp.exp2(s - m)
            il = 1.0 / jnp.sum(p, axis=0, keepdims=True)
            pn = p.astype(BF16)
            p_s[t, j] = pn
            vt = vT_s[pl.ds(pl.multiple_of(l0 + j * DH, DH), DH), pl.ds(q0, KW)]
            return _nn(vt, pn) * il, jnp.broadcast_to(il, (DH, QB))

        def fwd_step(t, tn, src, dst):
            qi, q0, l0 = idx(t)
            o_parts, il_parts = [], []
            for j in range(HG):
                qk_j(tn, dst, j)
                o, il = sm_pv_j(t, src, j)
                o_parts.append(o)
                il_parts.append(il)
            ot = jnp.concatenate(o_parts, axis=0)
            oT_s[t] = ot
            il_s[t] = jnp.concatenate(il_parts, axis=0)
            o_s[pl.ds(q0, QB), pl.ds(l0, 128)] = ot.T.astype(BF16)

        def fwd_body(i, c2):
            t = 2 * i
            fwd_step(t, t + 1, bufA, bufB)
            fwd_step(t + 1, jnp.minimum(t + 2, NT - 1), bufB, bufA)
            return c2

        with jax.named_scope("attn_fwd"):
            for j in range(HG):
                qk_j(0, bufA, j)
            lax.fori_loop(0, NT // 2, fwd_body, 0)

        rows = pl.ds(r0, SB)
        x = x_ref[rows, :].astype(F32)
        h = x + _nn(o_s[rows, :], wo_ref[...])
        y2, r2 = _ln(h)
        y2b = y2.astype(BF16)
        ln2_s[rows, :] = y2b
        gt = _nn(y2b, wg_ref[...])
        u = _nn(y2b, wu_ref[...])
        sg = jax.nn.sigmoid(gt)
        hh = (sg * u).astype(BF16)
        hh_s[rows, :] = hh
        out_ref[rows, :] = (h + _nn(hh, wd_ref[...])).astype(BF16)

        go = go_ref[rows, :]
        dhh = _nt(go, wd_ref[...])
        du = dhh * sg
        dg = du * u * (1.0 - sg)
        dub = du.astype(BF16)
        dgb = dg.astype(BF16)
        du_s[rows, :] = dub
        dg_s[rows, :] = dgb
        dy2 = _nt(dgb, wg_ref[...]) + _nt(dub, wu_ref[...])
        dh = go.astype(F32) + _ln_bwd(dy2, y2, r2)
        dh_s[rows, :] = dh
        doT_s[...] = _nt(wo_ref[...], dh.astype(BF16))

        def prep(t):
            b0 = pl.multiple_of((t // NG) * QB, QB)
            l0 = pl.multiple_of((t % NG) * 128, 128)
            dos = doT_s[pl.ds(l0, 128), pl.ds(b0, QB)] * il_s[t]
            return dos

        def dp_j(t, dos, dst, j):
            qi, q0, l0 = idx(t)
            vg = v_s[pl.ds(q0, KW), pl.ds(l0, 128)]
            wj = jnp.where(head_of_row == j, dos, 0.0).astype(BF16)
            dst[j] = _nn(vg, wj)

        def ds_j(t, dos, e, src, j):
            qi, q0, l0 = idx(t)
            hl = pl.ds(pl.multiple_of(l0 + j * DH, DH), DH)
            ej = jnp.sum(e[j * DH:(j + 1) * DH], axis=0, keepdims=True)
            pn = p_s[t, j]
            ds = (pn.astype(F32) * (src[j] - ej)).astype(BF16)
            dq = _nn(kT_s[hl, pl.ds(q0, KW)], ds)
            dkT_s[hl, pl.ds(q0, KW)] += _nt(qT_s[hl, pl.ds(q0, QB)], ds)
            dvT_s[hl, pl.ds(q0, KW)] += _nt(dos[j * DH:(j + 1) * DH].astype(BF16), pn)
            return dq

        def bwd_step(t, tn, src, dst):
            qi, q0, l0 = idx(t)
            dos = prep(t)
            e = dos * oT_s[t]
            dosn = prep(tn)
            parts = []
            for j in range(HG):
                dp_j(tn, dosn, dst, j)
                parts.append(ds_j(t, dos, e, src, j))
            dqt = jnp.concatenate(parts, axis=0) * SCALE
            dq_s[pl.ds(q0, QB), pl.ds(l0, 128)] = dqt.T.astype(BF16)

        def bwd_body(i, c2):
            t = 2 * i
            bwd_step(t, t + 1, bufA, bufB)
            bwd_step(t + 1, jnp.minimum(t + 2, NT - 1), bufB, bufA)
            return c2

        with jax.named_scope("attn_bwd"):
            dos0 = prep(0)
            for j in range(HG):
                dp_j(0, dos0, bufA, j)
            lax.fori_loop(0, NT // 2, bwd_body, 0)
        return carry

    with jax.named_scope("p2_all"):
        lax.fori_loop(0, NSB, p2, 0)

    def p3(c, carry):
        r0 = pl.multiple_of(c * RC, RC)
        rows = pl.ds(r0, RC)
        dqkv_s[rows, 0:D] = dq_s[rows, :]
        dqkv_s[rows, D:2 * D] = dkT_s[:, pl.ds(r0 + W, RC)].T.astype(BF16)
        dqkv_s[rows, 2 * D:3 * D] = dvT_s[:, pl.ds(r0 + W, RC)].T.astype(BF16)
        dy1 = _nt(dqkv_s[rows, :], wqkv_ref[...])
        x = x_ref[rows, :].astype(F32)
        y1, r1 = _ln(x)
        dx_ref[rows, :] = (dh_s[rows, :] + _ln_bwd(dy1, y1, r1)).astype(BF16)
        return carry

    with jax.named_scope("p3"):
        lax.fori_loop(0, S // RC, p3, 0)

    with jax.named_scope("p4_wgrad"):
        dwqkv_ref[...] = _tn(ln1_s[...], dqkv_s[...]).astype(BF16)
        dwo_ref[...] = _tn(o_s[...], dh_s[...].astype(BF16)).astype(BF16)
        dwg_ref[...] = _tn(ln2_s[...], dg_s[...]).astype(BF16)
        dwu_ref[...] = _tn(ln2_s[...], du_s[...]).astype(BF16)
        dwd_ref[...] = _tn(hh_s[...], go_ref[...]).astype(BF16)


@jax.jit
def pallas_sequential_preLN__sliding_block__glu_gated_glu__prompt_kernel(
    A_x: jax.Array,
    A_wqkv: jax.Array,
    A_wo: jax.Array,
    B_x: jax.Array,
    B_w_gate: jax.Array,
    B_w_up: jax.Array,
    B_w_down: jax.Array,
    grad_out: jax.Array,
):
    del B_x
    x = A_x.reshape(S, D)
    go = grad_out.reshape(S, D)
    sds = jax.ShapeDtypeStruct
    out_shape = (
        sds((S, D), BF16), sds((S, D), BF16),
        sds((D, 3 * D), BF16), sds((D, D), BF16),
        sds((D, F), BF16), sds((D, F), BF16), sds((F, D), BF16),
    )
    scratch = [
        pltpu.VMEM((S, D), BF16),
        pltpu.VMEM((S, D), BF16),
        pltpu.VMEM((D, S), BF16),
        pltpu.VMEM((S + W, D), BF16),
        pltpu.VMEM((D, S + W), BF16),
        pltpu.VMEM((S + W, D), BF16),
        pltpu.VMEM((D, S + W), BF16),
        pltpu.VMEM((S, D), BF16),
        pltpu.VMEM((NT, 128, QB), F32),
        pltpu.VMEM((NT, 128, QB), F32),
        pltpu.VMEM((NT, HG, KW, QB), BF16),
        pltpu.VMEM((D, SB), F32),
        pltpu.VMEM((S, D), BF16),
        pltpu.VMEM((S, F), BF16),
        pltpu.VMEM((S, F), BF16),
        pltpu.VMEM((S, F), BF16),
        pltpu.VMEM((S, D), F32),
        pltpu.VMEM((S, D), BF16),
        pltpu.VMEM((D, S + W), F32),
        pltpu.VMEM((D, S + W), F32),
        pltpu.VMEM((S, 3 * D), BF16),
        pltpu.VMEM((HG, KW, QB), F32),
        pltpu.VMEM((HG, KW, QB), F32),
        pltpu.VMEM((3, KW, QB), F32),
    ]
    outs = pl.pallas_call(
        _kernel,
        out_shape=out_shape,
        scratch_shapes=scratch,
        compiler_params=pltpu.CompilerParams(vmem_limit_bytes=120 * 1024 * 1024),
    )(x, A_wqkv, A_wo, B_w_gate, B_w_up, B_w_down, go)
    out, dx = outs[0].reshape(1, S, D), outs[1].reshape(1, S, D)
    return (out, dx) + tuple(outs[2:])
```

```python
import jax
import jax.numpy as jnp
from jax import lax
import jax.experimental.pallas as pl
import jax.experimental.pallas.tpu as pltpu

S, D, F = 2048, 512, 1376
H, DH, W = 32, 16, 256
QB = 128
KW = QB + W
NG = D // 128
HG = 128 // DH
SB = 256
NSB = S // SB
NT = (SB // QB) * NG
RC = 512
EPS = 1e-5
NEG = -1e9
SCALE = DH ** -0.5
LOG2E = 1.4426950408889634
F32 = jnp.float32
BF16 = jnp.bfloat16


def _nn(a, b):
    return jnp.dot(a, b, preferred_element_type=F32)


def _nt(a, b):
    return lax.dot_general(a, b, (((1,), (1,)), ((), ())), preferred_element_type=F32)


def _tn(a, b):
    return lax.dot_general(a, b, (((0,), (0,)), ((), ())), preferred_element_type=F32)


def _ln(x):
    m = jnp.mean(x, axis=-1, keepdims=True)
    xc = x - m
    v = jnp.mean(xc * xc, axis=-1, keepdims=True)
    r = lax.rsqrt(v + EPS)
    return xc * r, r


def _ln_bwd(dy, y, r):
    a = jnp.mean(dy, axis=-1, keepdims=True)
    b = jnp.mean(dy * y, axis=-1, keepdims=True)
    return r * (dy - a - y * b)


def _kernel(x_hbm, wqkv_hbm, wo_hbm, wg_hbm, wu_hbm, wd_hbm, go_hbm,
            out_hbm, dx_hbm, dwqkv_hbm, dwo_hbm, dwg_hbm, dwu_hbm, dwd_hbm,
            x_ref, wqkv_ref, wo_ref, wg_ref, wu_ref, wd_ref, go_ref,
            out_ref, dx_ref, dwqkv_ref, dwo_ref, dwg_ref, dwu_ref, dwd_ref,
            in_sems, out_sems, dx_sems, dw_sems,
            ln1_s, q_s, qT_s, k_s, kT_s, v_s, vT_s, o_s, oT_s, il_s, p_s, doT_s, ln2_s, hh_s,
            dg_s, du_s, dh_s, dq_s, dkT_s, dvT_s, dqkv_s, bufA, bufB, mb_s):
    in_pairs = [(x_hbm, x_ref), (wqkv_hbm, wqkv_ref), (wo_hbm, wo_ref), (wg_hbm, wg_ref),
                (wu_hbm, wu_ref), (wd_hbm, wd_ref), (go_hbm, go_ref)]
    in_copies = [pltpu.make_async_copy(src, dst, in_sems.at[i])
                 for i, (src, dst) in enumerate(in_pairs)]
    for cp in in_copies:
        cp.start()

    def out_copy(i):
        r = pl.ds(pl.multiple_of(i * SB, SB), SB)
        return pltpu.make_async_copy(out_ref.at[r, :], out_hbm.at[r, :], out_sems.at[i])

    def dx_copy(i):
        r = pl.ds(pl.multiple_of(i * RC, RC), RC)
        return pltpu.make_async_copy(dx_ref.at[r, :], dx_hbm.at[r, :], dx_sems.at[i])

    dw_pairs = [(dwqkv_ref, dwqkv_hbm), (dwg_ref, dwg_hbm), (dwu_ref, dwu_hbm),
                (dwd_ref, dwd_hbm), (dwo_ref, dwo_hbm)]
    dw_copies = [pltpu.make_async_copy(src, dst, dw_sems.at[i])
                 for i, (src, dst) in enumerate(dw_pairs)]

    k_s[0:W, :] = jnp.zeros((W, D), BF16)
    v_s[0:W, :] = jnp.zeros((W, D), BF16)
    kT_s[:, 0:W] = jnp.zeros((D, W), BF16)
    vT_s[:, 0:W] = jnp.zeros((D, W), BF16)
    dkT_s[...] = jnp.zeros(dkT_s.shape, F32)
    dvT_s[...] = jnp.zeros(dvT_s.shape, F32)

    c_i = lax.broadcasted_iota(jnp.int32, (KW, QB), 0)
    r_i = lax.broadcasted_iota(jnp.int32, (KW, QB), 1)
    for var in range(3):
        ok = (c_i > r_i) & (c_i <= r_i + W) & (c_i >= (2 - var) * QB)
        mb_s[var] = jnp.where(ok, 0.0, NEG)

    def p1(c, carry):
        r0 = pl.multiple_of(c * RC, RC)
        x = x_ref[pl.ds(r0, RC), :].astype(F32)
        y, _ = _ln(x)
        yb = y.astype(BF16)
        ln1_s[pl.ds(r0, RC), :] = yb
        qkv = _nn(yb, wqkv_ref[...])
        q = qkv[:, 0:D]
        k = qkv[:, D:2 * D]
        v = qkv[:, 2 * D:3 * D]
        q_s[pl.ds(r0, RC), :] = (q * (SCALE * LOG2E)).astype(BF16)
        k_s[pl.ds(r0 + W, RC), :] = k.astype(BF16)
        v_s[pl.ds(r0 + W, RC), :] = v.astype(BF16)
        qT_s[:, pl.ds(r0, RC)] = (q * SCALE).T.astype(BF16)
        kT_s[:, pl.ds(r0 + W, RC)] = k.T.astype(BF16)
        vT_s[:, pl.ds(r0 + W, RC)] = v.T.astype(BF16)
        return carry

    in_copies[0].wait()
    in_copies[1].wait()
    with jax.named_scope("p1_qkv"):
        lax.fori_loop(0, S // RC, p1, 0)
    for cp in in_copies[2:]:
        cp.wait()

    head_of_lane = lax.broadcasted_iota(jnp.int32, (QB, 128), 1) // DH
    head_of_row = lax.broadcasted_iota(jnp.int32, (128, QB), 0) // DH

    def p2(sb, carry):
        r0 = pl.multiple_of(sb * SB, SB)

        def idx(t):
            qi = sb * (SB // QB) + t // NG
            g = t % NG
            return qi, pl.multiple_of(qi * QB, QB), pl.multiple_of(g * 128, 128)

        def qk_j(t, dst, j):
            qi, q0, l0 = idx(t)
            qg = q_s[pl.ds(q0, QB), pl.ds(l0, 128)]
            kg = k_s[pl.ds(q0, KW), pl.ds(l0, 128)]
            qm = jnp.where(head_of_lane == j, qg, jnp.zeros_like(qg))
            dst[j] = _nt(kg, qm) + mb_s[jnp.minimum(qi, 2)]

        def sm_pv_j(t, src, j):
            qi, q0, l0 = idx(t)
            s = src[j]
            m = jnp.max(s, axis=0, keepdims=True)
            p = jnp.exp2(s - m)
            il = 1.0 / jnp.sum(p, axis=0, keepdims=True)
            pn = p.astype(BF16)
            p_s[t, j] = pn
            vt = vT_s[pl.ds(pl.multiple_of(l0 + j * DH, DH), DH), pl.ds(q0, KW)]
            return _nn(vt, pn) * il, jnp.broadcast_to(il, (DH, QB))

        def fwd_step(t, tn, src, dst):
            qi, q0, l0 = idx(t)
            o_parts, il_parts = [], []
            for j in range(HG):
                qk_j(tn, dst, j)
                o, il = sm_pv_j(t, src, j)
                o_parts.append(o)
                il_parts.append(il)
            ot = jnp.concatenate(o_parts, axis=0)
            oT_s[t] = ot
            il_s[t] = jnp.concatenate(il_parts, axis=0)
            o_s[pl.ds(q0, QB), pl.ds(l0, 128)] = ot.T.astype(BF16)

        def fwd_body(i, c2):
            t = 2 * i
            fwd_step(t, t + 1, bufA, bufB)
            fwd_step(t + 1, jnp.minimum(t + 2, NT - 1), bufB, bufA)
            return c2

        with jax.named_scope("attn_fwd"):
            for j in range(HG):
                qk_j(0, bufA, j)
            lax.fori_loop(0, NT // 2, fwd_body, 0)

        rows = pl.ds(r0, SB)
        x = x_ref[rows, :].astype(F32)
        h = x + _nn(o_s[rows, :], wo_ref[...])
        y2, r2 = _ln(h)
        y2b = y2.astype(BF16)
        ln2_s[rows, :] = y2b
        gt = _nn(y2b, wg_ref[...])
        u = _nn(y2b, wu_ref[...])
        sg = jax.nn.sigmoid(gt)
        hh = (sg * u).astype(BF16)
        hh_s[rows, :] = hh
        out_ref[rows, :] = (h + _nn(hh, wd_ref[...])).astype(BF16)
        out_copy(sb).start()

        go = go_ref[rows, :]
        dhh = _nt(go, wd_ref[...])
        du = dhh * sg
        dg = du * u * (1.0 - sg)
        dub = du.astype(BF16)
        dgb = dg.astype(BF16)
        du_s[rows, :] = dub
        dg_s[rows, :] = dgb
        dy2 = _nt(dgb, wg_ref[...]) + _nt(dub, wu_ref[...])
        dh = go.astype(F32) + _ln_bwd(dy2, y2, r2)
        dh_s[rows, :] = dh
        doT_s[...] = _nt(wo_ref[...], dh.astype(BF16))

        def prep(t):
            b0 = pl.multiple_of((t // NG) * QB, QB)
            l0 = pl.multiple_of((t % NG) * 128, 128)
            dos = doT_s[pl.ds(l0, 128), pl.ds(b0, QB)] * il_s[t]
            return dos

        def dp_j(t, dos, dst, j):
            qi, q0, l0 = idx(t)
            vg = v_s[pl.ds(q0, KW), pl.ds(l0, 128)]
            wj = jnp.where(head_of_row == j, dos, 0.0).astype(BF16)
            dst[j] = _nn(vg, wj)

        def ds_j(t, dos, e, src, j):
            qi, q0, l0 = idx(t)
            hl = pl.ds(pl.multiple_of(l0 + j * DH, DH), DH)
            ej = jnp.sum(e[j * DH:(j + 1) * DH], axis=0, keepdims=True)
            pn = p_s[t, j]
            ds = (pn.astype(F32) * (src[j] - ej)).astype(BF16)
            dq = _nn(kT_s[hl, pl.ds(q0, KW)], ds)
            dkT_s[hl, pl.ds(q0, KW)] += _nt(qT_s[hl, pl.ds(q0, QB)], ds)
            dvT_s[hl, pl.ds(q0, KW)] += _nt(dos[j * DH:(j + 1) * DH].astype(BF16), pn)
            return dq

        def bwd_step(t, tn, src, dst):
            qi, q0, l0 = idx(t)
            dos = prep(t)
            e = dos * oT_s[t]
            dosn = prep(tn)
            parts = []
            for j in range(HG):
                dp_j(tn, dosn, dst, j)
                parts.append(ds_j(t, dos, e, src, j))
            dqt = jnp.concatenate(parts, axis=0) * SCALE
            dq_s[pl.ds(q0, QB), pl.ds(l0, 128)] = dqt.T.astype(BF16)

        def bwd_body(i, c2):
            t = 2 * i
            bwd_step(t, t + 1, bufA, bufB)
            bwd_step(t + 1, jnp.minimum(t + 2, NT - 1), bufB, bufA)
            return c2

        with jax.named_scope("attn_bwd"):
            dos0 = prep(0)
            for j in range(HG):
                dp_j(0, dos0, bufA, j)
            lax.fori_loop(0, NT // 2, bwd_body, 0)
        return carry

    with jax.named_scope("p2_all"):
        lax.fori_loop(0, NSB, p2, 0)

    def p3(c, carry):
        r0 = pl.multiple_of(c * RC, RC)
        rows = pl.ds(r0, RC)
        dqkv_s[rows, 0:D] = dq_s[rows, :]
        dqkv_s[rows, D:2 * D] = dkT_s[:, pl.ds(r0 + W, RC)].T.astype(BF16)
        dqkv_s[rows, 2 * D:3 * D] = dvT_s[:, pl.ds(r0 + W, RC)].T.astype(BF16)
        dy1 = _nt(dqkv_s[rows, :], wqkv_ref[...])
        x = x_ref[rows, :].astype(F32)
        y1, r1 = _ln(x)
        dx_ref[rows, :] = (dh_s[rows, :] + _ln_bwd(dy1, y1, r1)).astype(BF16)
        dx_copy(c).start()
        return carry

    with jax.named_scope("p3"):
        lax.fori_loop(0, S // RC, p3, 0)

    with jax.named_scope("p4_wgrad"):
        dwqkv_ref[...] = _tn(ln1_s[...], dqkv_s[...]).astype(BF16)
        dw_copies[0].start()
        dwg_ref[...] = _tn(ln2_s[...], dg_s[...]).astype(BF16)
        dw_copies[1].start()
        dwu_ref[...] = _tn(ln2_s[...], du_s[...]).astype(BF16)
        dw_copies[2].start()
        dwd_ref[...] = _tn(hh_s[...], go_ref[...]).astype(BF16)
        dw_copies[3].start()
        dwo_ref[...] = _tn(o_s[...], dh_s[...].astype(BF16)).astype(BF16)
        dw_copies[4].start()
    for i in range(NSB):
        out_copy(i).wait()
    for i in range(S // RC):
        dx_copy(i).wait()
    for cp in dw_copies:
        cp.wait()


@jax.jit
def pallas_sequential_preLN__sliding_block__glu_gated_glu__prompt_kernel(
    A_x: jax.Array,
    A_wqkv: jax.Array,
    A_wo: jax.Array,
    B_x: jax.Array,
    B_w_gate: jax.Array,
    B_w_up: jax.Array,
    B_w_down: jax.Array,
    grad_out: jax.Array,
):
    del B_x
    x = A_x.reshape(S, D)
    go = grad_out.reshape(S, D)
    sds = jax.ShapeDtypeStruct
    out_shape = (
        sds((S, D), BF16), sds((S, D), BF16),
        sds((D, 3 * D), BF16), sds((D, D), BF16),
        sds((D, F), BF16), sds((D, F), BF16), sds((F, D), BF16),
    )
    scratch = [
        pltpu.VMEM((S, D), BF16), pltpu.VMEM((D, 3 * D), BF16), pltpu.VMEM((D, D), BF16),
        pltpu.VMEM((D, F), BF16), pltpu.VMEM((D, F), BF16), pltpu.VMEM((F, D), BF16),
        pltpu.VMEM((S, D), BF16),
        pltpu.VMEM((S, D), BF16), pltpu.VMEM((S, D), BF16),
        pltpu.VMEM((D, 3 * D), BF16), pltpu.VMEM((D, D), BF16),
        pltpu.VMEM((D, F), BF16), pltpu.VMEM((D, F), BF16), pltpu.VMEM((F, D), BF16),
        pltpu.SemaphoreType.DMA((7,)), pltpu.SemaphoreType.DMA((NSB,)),
        pltpu.SemaphoreType.DMA((S // RC,)), pltpu.SemaphoreType.DMA((5,)),
        pltpu.VMEM((S, D), BF16),
        pltpu.VMEM((S, D), BF16),
        pltpu.VMEM((D, S), BF16),
        pltpu.VMEM((S + W, D), BF16),
        pltpu.VMEM((D, S + W), BF16),
        pltpu.VMEM((S + W, D), BF16),
        pltpu.VMEM((D, S + W), BF16),
        pltpu.VMEM((S, D), BF16),
        pltpu.VMEM((NT, 128, QB), F32),
        pltpu.VMEM((NT, 128, QB), F32),
        pltpu.VMEM((NT, HG, KW, QB), BF16),
        pltpu.VMEM((D, SB), F32),
        pltpu.VMEM((S, D), BF16),
        pltpu.VMEM((S, F), BF16),
        pltpu.VMEM((S, F), BF16),
        pltpu.VMEM((S, F), BF16),
        pltpu.VMEM((S, D), F32),
        pltpu.VMEM((S, D), BF16),
        pltpu.VMEM((D, S + W), F32),
        pltpu.VMEM((D, S + W), F32),
        pltpu.VMEM((S, 3 * D), BF16),
        pltpu.VMEM((HG, KW, QB), F32),
        pltpu.VMEM((HG, KW, QB), F32),
        pltpu.VMEM((3, KW, QB), F32),
    ]
    outs = pl.pallas_call(
        _kernel,
        out_shape=out_shape,
        in_specs=[pl.BlockSpec(memory_space=pl.ANY)] * 7,
        out_specs=tuple(pl.BlockSpec(memory_space=pl.ANY) for _ in range(7)),
        scratch_shapes=scratch,
        compiler_params=pltpu.CompilerParams(vmem_limit_bytes=120 * 1024 * 1024),
    )(x, A_wqkv, A_wo, B_w_gate, B_w_up, B_w_down, go)
    out, dx = outs[0].reshape(1, S, D), outs[1].reshape(1, S, D)
    return (out, dx) + tuple(outs[2:])
```

```python
import jax
import jax.numpy as jnp
from jax import lax
import jax.experimental.pallas as pl
import jax.experimental.pallas.tpu as pltpu

S, D, F = 2048, 512, 1376
H, DH, W = 32, 16, 256
QB = 128
KW = QB + W
NG = D // 128
HG = 128 // DH
SB = 256
NSB = S // SB
NT = (SB // QB) * NG
RC = 512
EPS = 1e-5
NEG = -1e9
SCALE = DH ** -0.5
LOG2E = 1.4426950408889634
F32 = jnp.float32
BF16 = jnp.bfloat16


def _nn(a, b):
    return jnp.dot(a, b, preferred_element_type=F32)


def _nt(a, b):
    return lax.dot_general(a, b, (((1,), (1,)), ((), ())), preferred_element_type=F32)


def _tn(a, b):
    return lax.dot_general(a, b, (((0,), (0,)), ((), ())), preferred_element_type=F32)


def _ln(x):
    m = jnp.mean(x, axis=-1, keepdims=True)
    xc = x - m
    v = jnp.mean(xc * xc, axis=-1, keepdims=True)
    r = lax.rsqrt(v + EPS)
    return xc * r, r


def _ln_bwd(dy, y, r):
    a = jnp.mean(dy, axis=-1, keepdims=True)
    b = jnp.mean(dy * y, axis=-1, keepdims=True)
    return r * (dy - a - y * b)


def _kernel(x_hbm, wqkv_hbm, wo_hbm, wg_hbm, wu_hbm, wd_hbm, go_hbm,
            out_hbm, dx_hbm, dwqkv_hbm, dwo_hbm, dwg_hbm, dwu_hbm, dwd_hbm,
            x_ref, wqkv_ref, wo_ref, wg_ref, wu_ref, wd_ref, go_ref,
            out_ref, dx_ref, dwqkv_ref, dwo_ref, dwg_ref, dwu_ref, dwd_ref,
            in_sems, out_sems, dx_sems, dw_sems,
            ln1_s, q_s, qT_s, k_s, kT_s, v_s, vT_s, o_s, oT_s, il_s, p_s, doT_s, ln2_s, hh_s,
            dg_s, du_s, dh_s, dq_s, dkT_s, dvT_s, dqkv_s, bufA, bufB, mb_s):
    in_pairs = [(x_hbm, x_ref), (wqkv_hbm, wqkv_ref), (wo_hbm, wo_ref), (wg_hbm, wg_ref),
                (wu_hbm, wu_ref), (wd_hbm, wd_ref), (go_hbm, go_ref)]
    in_copies = [pltpu.make_async_copy(src, dst, in_sems.at[i])
                 for i, (src, dst) in enumerate(in_pairs)]
    for cp in in_copies:
        cp.start()

    def out_copy(i):
        r = pl.ds(pl.multiple_of(i * SB, SB), SB)
        return pltpu.make_async_copy(out_ref.at[r, :], out_hbm.at[r, :], out_sems.at[i])

    def dx_copy(i):
        r = pl.ds(pl.multiple_of(i * RC, RC), RC)
        return pltpu.make_async_copy(dx_ref.at[r, :], dx_hbm.at[r, :], dx_sems.at[i])

    dw_pairs = [(dwqkv_ref, dwqkv_hbm), (dwg_ref, dwg_hbm), (dwu_ref, dwu_hbm),
                (dwd_ref, dwd_hbm), (dwo_ref, dwo_hbm)]
    dw_copies = [pltpu.make_async_copy(src, dst, dw_sems.at[i])
                 for i, (src, dst) in enumerate(dw_pairs)]

    k_s[0:W, :] = jnp.zeros((W, D), BF16)
    v_s[0:W, :] = jnp.zeros((W, D), BF16)
    kT_s[:, 0:W] = jnp.zeros((D, W), BF16)
    vT_s[:, 0:W] = jnp.zeros((D, W), BF16)
    dkT_s[...] = jnp.zeros(dkT_s.shape, F32)
    dvT_s[...] = jnp.zeros(dvT_s.shape, F32)

    c_i = lax.broadcasted_iota(jnp.int32, (KW, QB), 0)
    r_i = lax.broadcasted_iota(jnp.int32, (KW, QB), 1)
    for var in range(3):
        ok = (c_i > r_i) & (c_i <= r_i + W) & (c_i >= (2 - var) * QB)
        mb_s[var] = jnp.where(ok, 0.0, NEG)

    def p1(c, carry):
        r0 = pl.multiple_of(c * RC, RC)
        x = x_ref[pl.ds(r0, RC), :].astype(F32)
        y, _ = _ln(x)
        yb = y.astype(BF16)
        ln1_s[pl.ds(r0, RC), :] = yb
        qkv = _nn(yb, wqkv_ref[...])
        q = qkv[:, 0:D]
        k = qkv[:, D:2 * D]
        v = qkv[:, 2 * D:3 * D]
        q_s[pl.ds(r0, RC), :] = (q * (SCALE * LOG2E)).astype(BF16)
        k_s[pl.ds(r0 + W, RC), :] = k.astype(BF16)
        v_s[pl.ds(r0 + W, RC), :] = v.astype(BF16)
        qT_s[:, pl.ds(r0, RC)] = (q * SCALE).T.astype(BF16)
        kT_s[:, pl.ds(r0 + W, RC)] = k.T.astype(BF16)
        vT_s[:, pl.ds(r0 + W, RC)] = v.T.astype(BF16)
        return carry

    in_copies[0].wait()
    in_copies[1].wait()
    with jax.named_scope("p1_qkv"):
        lax.fori_loop(0, S // RC, p1, 0)
    for cp in in_copies[2:]:
        cp.wait()

    head_of_lane = lax.broadcasted_iota(jnp.int32, (QB, 128), 1) // DH
    head_of_row = lax.broadcasted_iota(jnp.int32, (128, QB), 0) // DH

    def p2(sb, carry):
        r0 = pl.multiple_of(sb * SB, SB)

        def idx(t):
            qi = sb * (SB // QB) + t // NG
            g = t % NG
            return qi, pl.multiple_of(qi * QB, QB), pl.multiple_of(g * 128, 128)

        def qk_j(t, dst, j):
            qi, q0, l0 = idx(t)
            qg = q_s[pl.ds(q0, QB), pl.ds(l0, 128)]
            kg = k_s[pl.ds(q0, KW), pl.ds(l0, 128)]
            qm = jnp.where(head_of_lane == j, qg, jnp.zeros_like(qg))
            dst[j] = _nt(kg, qm) + mb_s[jnp.minimum(qi, 2)]

        def sm_pv_j(t, src, j):
            qi, q0, l0 = idx(t)
            s = src[j]
            m = jnp.max(s, axis=0, keepdims=True)
            p = jnp.exp2(s - m)
            il = 1.0 / jnp.sum(p, axis=0, keepdims=True)
            pn = p.astype(BF16)
            p_s[t, j] = pn
            vt = vT_s[pl.ds(pl.multiple_of(l0 + j * DH, DH), DH), pl.ds(q0, KW)]
            return _nn(vt, pn) * il, jnp.broadcast_to(il, (DH, QB))

        def fwd_step(t, tn, src, dst):
            qi, q0, l0 = idx(t)
            o_parts, il_parts = [], []
            for j in range(HG):
                qk_j(tn, dst, j)
                o, il = sm_pv_j(t, src, j)
                o_parts.append(o)
                il_parts.append(il)
            ot = jnp.concatenate(o_parts, axis=0)
            oT_s[t] = ot
            il_s[t] = jnp.concatenate(il_parts, axis=0)
            o_s[pl.ds(q0, QB), pl.ds(l0, 128)] = ot.T.astype(BF16)

        def fwd_body(i, c2):
            t = 2 * i
            fwd_step(t, t + 1, bufA, bufB)
            fwd_step(t + 1, jnp.minimum(t + 2, NT - 1), bufB, bufA)
            return c2

        with jax.named_scope("attn_fwd"):
            for j in range(HG):
                qk_j(0, bufA, j)
            lax.fori_loop(0, NT // 2, fwd_body, 0)

        rows = pl.ds(r0, SB)
        x = x_ref[rows, :].astype(F32)
        h = x + _nn(o_s[rows, :], wo_ref[...])
        y2, r2 = _ln(h)
        y2b = y2.astype(BF16)
        ln2_s[rows, :] = y2b
        gt = _nt(y2b, wg_ref[...])
        u = _nt(y2b, wu_ref[...])
        sg = jax.nn.sigmoid(gt)
        hh = (sg * u).astype(BF16)
        hh_s[rows, :] = hh
        out_ref[rows, :] = (h + _nn(hh, wd_ref[...])).astype(BF16)
        out_copy(sb).start()

        go = go_ref[rows, :]
        dhh = _nt(go, wd_ref[...])
        du = dhh * sg
        dg = du * u * (1.0 - sg)
        dub = du.astype(BF16)
        dgb = dg.astype(BF16)
        du_s[rows, :] = dub
        dg_s[rows, :] = dgb
        dy2 = _nn(dgb, wg_ref[...]) + _nn(dub, wu_ref[...])
        dh = go.astype(F32) + _ln_bwd(dy2, y2, r2)
        dh_s[rows, :] = dh
        doT_s[...] = _nt(wo_ref[...], dh.astype(BF16))

        def prep(t):
            b0 = pl.multiple_of((t // NG) * QB, QB)
            l0 = pl.multiple_of((t % NG) * 128, 128)
            dos = doT_s[pl.ds(l0, 128), pl.ds(b0, QB)] * il_s[t]
            return dos

        def dp_j(t, dos, dst, j):
            qi, q0, l0 = idx(t)
            vg = v_s[pl.ds(q0, KW), pl.ds(l0, 128)]
            wj = jnp.where(head_of_row == j, dos, 0.0).astype(BF16)
            dst[j] = _nn(vg, wj)

        def ds_j(t, dos, e, src, j):
            qi, q0, l0 = idx(t)
            hl = pl.ds(pl.multiple_of(l0 + j * DH, DH), DH)
            ej = jnp.sum(e[j * DH:(j + 1) * DH], axis=0, keepdims=True)
            pn = p_s[t, j]
            ds = (pn.astype(F32) * (src[j] - ej)).astype(BF16)
            dq = _nn(kT_s[hl, pl.ds(q0, KW)], ds)
            dkT_s[hl, pl.ds(q0, KW)] += _nt(qT_s[hl, pl.ds(q0, QB)], ds)
            dvT_s[hl, pl.ds(q0, KW)] += _nt(dos[j * DH:(j + 1) * DH].astype(BF16), pn)
            return dq

        def bwd_step(t, tn, src, dst):
            qi, q0, l0 = idx(t)
            dos = prep(t)
            e = dos * oT_s[t]
            dosn = prep(tn)
            parts = []
            for j in range(HG):
                dp_j(tn, dosn, dst, j)
                parts.append(ds_j(t, dos, e, src, j))
            dqt = jnp.concatenate(parts, axis=0) * SCALE
            dq_s[pl.ds(q0, QB), pl.ds(l0, 128)] = dqt.T.astype(BF16)

        def bwd_body(i, c2):
            t = 2 * i
            bwd_step(t, t + 1, bufA, bufB)
            bwd_step(t + 1, jnp.minimum(t + 2, NT - 1), bufB, bufA)
            return c2

        with jax.named_scope("attn_bwd"):
            dos0 = prep(0)
            for j in range(HG):
                dp_j(0, dos0, bufA, j)
            lax.fori_loop(0, NT // 2, bwd_body, 0)
        return carry

    with jax.named_scope("p2_all"):
        lax.fori_loop(0, NSB, p2, 0)

    def p3(c, carry):
        r0 = pl.multiple_of(c * RC, RC)
        rows = pl.ds(r0, RC)
        dqkv_s[rows, 0:D] = dq_s[rows, :]
        dqkv_s[rows, D:2 * D] = dkT_s[:, pl.ds(r0 + W, RC)].T.astype(BF16)
        dqkv_s[rows, 2 * D:3 * D] = dvT_s[:, pl.ds(r0 + W, RC)].T.astype(BF16)
        dy1 = _nt(dqkv_s[rows, :], wqkv_ref[...])
        x = x_ref[rows, :].astype(F32)
        y1, r1 = _ln(x)
        dx_ref[rows, :] = (dh_s[rows, :] + _ln_bwd(dy1, y1, r1)).astype(BF16)
        dx_copy(c).start()
        return carry

    with jax.named_scope("p3"):
        lax.fori_loop(0, S // RC, p3, 0)

    with jax.named_scope("p4_wgrad"):
        dwqkv_ref[...] = _tn(ln1_s[...], dqkv_s[...]).astype(BF16)
        dw_copies[0].start()
        dwg_ref[...] = _tn(dg_s[...], ln2_s[...]).astype(BF16)
        dw_copies[1].start()
        dwu_ref[...] = _tn(du_s[...], ln2_s[...]).astype(BF16)
        dw_copies[2].start()
        dwd_ref[...] = _tn(hh_s[...], go_ref[...]).astype(BF16)
        dw_copies[3].start()
        dwo_ref[...] = _tn(o_s[...], dh_s[...].astype(BF16)).astype(BF16)
        dw_copies[4].start()
    for i in range(NSB):
        out_copy(i).wait()
    for i in range(S // RC):
        dx_copy(i).wait()
    for cp in dw_copies:
        cp.wait()


@jax.jit
def pallas_sequential_preLN__sliding_block__glu_gated_glu__prompt_kernel(
    A_x: jax.Array,
    A_wqkv: jax.Array,
    A_wo: jax.Array,
    B_x: jax.Array,
    B_w_gate: jax.Array,
    B_w_up: jax.Array,
    B_w_down: jax.Array,
    grad_out: jax.Array,
):
    del B_x
    x = A_x.reshape(S, D)
    go = grad_out.reshape(S, D)
    sds = jax.ShapeDtypeStruct
    out_shape = (
        sds((S, D), BF16), sds((S, D), BF16),
        sds((D, 3 * D), BF16), sds((D, D), BF16),
        sds((F, D), BF16), sds((F, D), BF16), sds((F, D), BF16),
    )
    scratch = [
        pltpu.VMEM((S, D), BF16), pltpu.VMEM((D, 3 * D), BF16), pltpu.VMEM((D, D), BF16),
        pltpu.VMEM((F, D), BF16), pltpu.VMEM((F, D), BF16), pltpu.VMEM((F, D), BF16),
        pltpu.VMEM((S, D), BF16),
        pltpu.VMEM((S, D), BF16), pltpu.VMEM((S, D), BF16),
        pltpu.VMEM((D, 3 * D), BF16), pltpu.VMEM((D, D), BF16),
        pltpu.VMEM((F, D), BF16), pltpu.VMEM((F, D), BF16), pltpu.VMEM((F, D), BF16),
        pltpu.SemaphoreType.DMA((7,)), pltpu.SemaphoreType.DMA((NSB,)),
        pltpu.SemaphoreType.DMA((S // RC,)), pltpu.SemaphoreType.DMA((5,)),
        pltpu.VMEM((S, D), BF16),
        pltpu.VMEM((S, D), BF16),
        pltpu.VMEM((D, S), BF16),
        pltpu.VMEM((S + W, D), BF16),
        pltpu.VMEM((D, S + W), BF16),
        pltpu.VMEM((S + W, D), BF16),
        pltpu.VMEM((D, S + W), BF16),
        pltpu.VMEM((S, D), BF16),
        pltpu.VMEM((NT, 128, QB), F32),
        pltpu.VMEM((NT, 128, QB), F32),
        pltpu.VMEM((NT, HG, KW, QB), BF16),
        pltpu.VMEM((D, SB), F32),
        pltpu.VMEM((S, D), BF16),
        pltpu.VMEM((S, F), BF16),
        pltpu.VMEM((S, F), BF16),
        pltpu.VMEM((S, F), BF16),
        pltpu.VMEM((S, D), F32),
        pltpu.VMEM((S, D), BF16),
        pltpu.VMEM((D, S + W), F32),
        pltpu.VMEM((D, S + W), F32),
        pltpu.VMEM((S, 3 * D), BF16),
        pltpu.VMEM((HG, KW, QB), F32),
        pltpu.VMEM((HG, KW, QB), F32),
        pltpu.VMEM((3, KW, QB), F32),
    ]
    outs = pl.pallas_call(
        _kernel,
        out_shape=out_shape,
        in_specs=[pl.BlockSpec(memory_space=pl.ANY)] * 7,
        out_specs=tuple(pl.BlockSpec(memory_space=pl.ANY) for _ in range(7)),
        scratch_shapes=scratch,
        compiler_params=pltpu.CompilerParams(vmem_limit_bytes=120 * 1024 * 1024),
    )(x, A_wqkv, A_wo, B_w_gate.T, B_w_up.T, B_w_down, go)
    out, dx = outs[0].reshape(1, S, D), outs[1].reshape(1, S, D)
    return (out, dx, outs[2], outs[3], outs[4].T, outs[5].T, outs[6])
```

```python
import jax
import jax.numpy as jnp
from jax import lax
import jax.experimental.pallas as pl
import jax.experimental.pallas.tpu as pltpu

S, D, F = 2048, 512, 1376
H, DH, W = 32, 16, 256
NG = D // 128
HP = 2
QP = 128 // HP
KP = QP + W
NU = 8 // HP
UL = HP * DH
NVAR = W // QP + 1
SB = 256
NSB = S // SB
NT = (SB // QP) * NG
RC = 512
PADT = 128
EPS = 1e-5
NEG = -1e9
SCALE = DH ** -0.5
LOG2E = 1.4426950408889634
F32 = jnp.float32
BF16 = jnp.bfloat16


def _nn(a, b):
    return jnp.dot(a, b, preferred_element_type=F32)


def _nt(a, b):
    return lax.dot_general(a, b, (((1,), (1,)), ((), ())), preferred_element_type=F32)


def _tn(a, b):
    return lax.dot_general(a, b, (((0,), (0,)), ((), ())), preferred_element_type=F32)


def _ln(x):
    m = jnp.mean(x, axis=-1, keepdims=True)
    xc = x - m
    v = jnp.mean(xc * xc, axis=-1, keepdims=True)
    r = lax.rsqrt(v + EPS)
    return xc * r, r


def _ln_bwd(dy, y, r):
    a = jnp.mean(dy, axis=-1, keepdims=True)
    b = jnp.mean(dy * y, axis=-1, keepdims=True)
    return r * (dy - a - y * b)


def _kernel(x_hbm, wqkv_hbm, wo_hbm, wg_hbm, wu_hbm, wd_hbm, go_hbm,
            out_hbm, dx_hbm, dwqkv_hbm, dwo_hbm, dwg_hbm, dwu_hbm, dwd_hbm,
            x_ref, wqkv_ref, wo_ref, wg_ref, wu_ref, wd_ref, go_ref,
            out_ref, dx_ref, dwqkv_ref, dwo_ref, dwg_ref, dwu_ref, dwd_ref,
            in_sems, out_sems, dx_sems, dw_sems,
            ln1_s, q_s, k_s, kT_s, v_s, vT_s, o_s, oT_s, il_s, p_s, do_s, ln2_s, hh_s,
            dg_s, du_s, dh_s, dq_s, dkT_s, dvT_s, dqkv_s, bufA, bufB, mb_s):
    in_pairs = [(x_hbm, x_ref), (wqkv_hbm, wqkv_ref), (wo_hbm, wo_ref), (wg_hbm, wg_ref),
                (wu_hbm, wu_ref), (wd_hbm, wd_ref), (go_hbm, go_ref)]
    in_copies = [pltpu.make_async_copy(src, dst, in_sems.at[i])
                 for i, (src, dst) in enumerate(in_pairs)]
    for cp in in_copies:
        cp.start()

    def out_copy(i):
        r = pl.ds(pl.multiple_of(i * SB, SB), SB)
        return pltpu.make_async_copy(out_ref.at[r, :], out_hbm.at[r, :], out_sems.at[i])

    def dx_copy(i):
        r = pl.ds(pl.multiple_of(i * RC, RC), RC)
        return pltpu.make_async_copy(dx_ref.at[r, :], dx_hbm.at[r, :], dx_sems.at[i])

    dw_pairs = [(dwqkv_ref, dwqkv_hbm), (dwg_ref, dwg_hbm), (dwu_ref, dwu_hbm),
                (dwd_ref, dwd_hbm), (dwo_ref, dwo_hbm)]
    dw_copies = [pltpu.make_async_copy(src, dst, dw_sems.at[i])
                 for i, (src, dst) in enumerate(dw_pairs)]

    k_s[0:W, :] = jnp.zeros((W, D), BF16)
    v_s[0:W, :] = jnp.zeros((W, D), BF16)
    k_s[S + W:, :] = jnp.zeros((PADT, D), BF16)
    v_s[S + W:, :] = jnp.zeros((PADT, D), BF16)
    kT_s[0, :, 0:W] = jnp.zeros((D, W), BF16)
    vT_s[0, :, 0:W] = jnp.zeros((D, W), BF16)
    dkT_s[...] = jnp.zeros(dkT_s.shape, F32)
    dvT_s[...] = jnp.zeros(dvT_s.shape, F32)

    c_i = lax.broadcasted_iota(jnp.int32, (KP, 128), 0)
    r_i = lax.broadcasted_iota(jnp.int32, (KP, 128), 1) % QP
    for var in range(NVAR):
        ok = (c_i > r_i) & (c_i <= r_i + W) & (c_i >= W - var * QP)
        mb_s[var] = jnp.where(ok, 0.0, NEG)

    def p1(c, carry):
        r0 = pl.multiple_of(c * RC, RC)
        x = x_ref[pl.ds(r0, RC), :].astype(F32)
        y, _ = _ln(x)
        yb = y.astype(BF16)
        ln1_s[pl.ds(r0, RC), :] = yb
        qkv = _nn(yb, wqkv_ref[...])
        k = qkv[:, D:2 * D]
        v = qkv[:, 2 * D:3 * D]
        q_s[pl.ds(r0, RC), :] = (qkv[:, 0:D] * (SCALE * LOG2E)).astype(BF16)
        k_s[pl.ds(r0 + W, RC), :] = k.astype(BF16)
        v_s[pl.ds(r0 + W, RC), :] = v.astype(BF16)
        kT_s[0, :, pl.ds(r0 + W, RC)] = k.T.astype(BF16)
        vT_s[0, :, pl.ds(r0 + W, RC)] = v.T.astype(BF16)
        return carry

    def p1b(c, carry):
        a = pl.multiple_of(c * 256, 256)
        kT_s[1, :, pl.ds(a, 256)] = k_s[pl.ds(a + QP, 256), :].T
        vT_s[1, :, pl.ds(a, 256)] = v_s[pl.ds(a + QP, 256), :].T
        return carry

    in_copies[0].wait()
    in_copies[1].wait()
    with jax.named_scope("p1_qkv"):
        lax.fori_loop(0, S // RC, p1, 0)
        lax.fori_loop(0, (S + W) // 256, p1b, 0)
    for cp in in_copies[2:]:
        cp.wait()

    head_of_lane = lax.broadcasted_iota(jnp.int32, (QP, 128), 1) // DH
    slot_of_lane = head_of_lane % HP
    unit_of_row = lax.broadcasted_iota(jnp.int32, (128, 128), 0) // UL

    def spread(t, sel):
        z = jnp.zeros_like(t)
        return jnp.concatenate([jnp.where(sel(hp), t, z) for hp in range(HP)], axis=0)

    def gather(t):
        r = t[0:QP]
        for hp in range(1, HP):
            r = jnp.where(slot_of_lane == hp, t[hp * QP:(hp + 1) * QP], r)
        return r

    def p2(sb, carry):
        r0 = pl.multiple_of(sb * SB, SB)

        def idx(t):
            qi = sb * (SB // QP) + t // NG
            g = t % NG
            return qi, pl.multiple_of(qi * QP, QP), pl.multiple_of(g * 128, 128)

        def tidx(t):
            qi = sb * (SB // QP) + t // NG
            return qi % 2, pl.multiple_of((qi // 2) * 128, 128)

        def qk_u(t, dst, u):
            qi, q0, l0 = idx(t)
            qg = q_s[pl.ds(q0, QP), pl.ds(l0, 128)]
            kg = k_s[pl.ds(q0, KP), pl.ds(l0, 128)]
            qm = spread(qg, lambda hp: head_of_lane == u * HP + hp)
            dst[u] = _nt(kg, qm) + mb_s[jnp.minimum(qi, NVAR - 1)]

        def sm_pv_u(t, src, u):
            qi, q0, l0 = idx(t)
            s = src[u]
            m = jnp.max(s, axis=0, keepdims=True)
            p = jnp.exp2(s - m)
            il = 1.0 / jnp.sum(p, axis=0, keepdims=True)
            pn = p.astype(BF16)
            p_s[t, u] = pn
            par, a0 = tidx(t)
            vt = vT_s[par, pl.ds(pl.multiple_of(l0 + u * UL, UL), UL), pl.ds(a0, KP)]
            return _nn(vt, pn) * il, jnp.broadcast_to(il, (UL, 128))

        def fwd_step(t, tn, src, dst):
            qi, q0, l0 = idx(t)
            o_parts, il_parts = [], []
            for u in range(NU):
                qk_u(tn, dst, u)
                o, il = sm_pv_u(t, src, u)
                o_parts.append(o)
                il_parts.append(il)
            ot = jnp.concatenate(o_parts, axis=0)
            oT_s[t] = ot
            il_s[t] = jnp.concatenate(il_parts, axis=0)
            o_s[pl.ds(q0, QP), pl.ds(l0, 128)] = gather(ot.T).astype(BF16)

        def fwd_body(i, c2):
            t = 2 * i
            fwd_step(t, t + 1, bufA, bufB)
            fwd_step(t + 1, jnp.minimum(t + 2, NT - 1), bufB, bufA)
            return c2

        with jax.named_scope("attn_fwd"):
            for u in range(NU):
                qk_u(0, bufA, u)
            lax.fori_loop(0, NT // 2, fwd_body, 0)

        rows = pl.ds(r0, SB)
        x = x_ref[rows, :].astype(F32)
        h = x + _nn(o_s[rows, :], wo_ref[...])
        y2, r2 = _ln(h)
        y2b = y2.astype(BF16)
        ln2_s[rows, :] = y2b
        gt = _nt(y2b, wg_ref[...])
        u_ = _nt(y2b, wu_ref[...])
        sg = jax.nn.sigmoid(gt)
        hh = (sg * u_).astype(BF16)
        hh_s[rows, :] = hh
        out_ref[rows, :] = (h + _nn(hh, wd_ref[...])).astype(BF16)
        out_copy(sb).start()

        go = go_ref[rows, :]
        dhh = _nt(go, wd_ref[...])
        du = dhh * sg
        dg = du * u_ * (1.0 - sg)
        dub = du.astype(BF16)
        dgb = dg.astype(BF16)
        du_s[rows, :] = dub
        dg_s[rows, :] = dgb
        dy2 = _nn(dgb, wg_ref[...]) + _nn(dub, wu_ref[...])
        dh = go.astype(F32) + _ln_bwd(dy2, y2, r2)
        dh_s[rows, :] = dh
        do_s[...] = _nt(dh.astype(BF16), wo_ref[...])

        def prep(t):
            b0 = pl.multiple_of((t // NG) * QP, QP)
            l0 = pl.multiple_of((t % NG) * 128, 128)
            dog = do_s[pl.ds(b0, QP), pl.ds(l0, 128)]
            return spread(dog, lambda hp: slot_of_lane == hp).T * il_s[t]

        def dp_u(t, dos, dst, u):
            qi, q0, l0 = idx(t)
            vg = v_s[pl.ds(q0, KP), pl.ds(l0, 128)]
            wj = jnp.where(unit_of_row == u, dos, 0.0).astype(BF16)
            dst[u] = _nn(vg, wj)

        def ds_u(t, dos, e, qbd, src, u):
            qi, q0, l0 = idx(t)
            hl = pl.ds(pl.multiple_of(l0 + u * UL, UL), UL)
            eu = jnp.sum(e[u * UL:(u + 1) * UL], axis=0, keepdims=True)
            pn = p_s[t, u]
            ds = (pn.astype(F32) * (src[u] - eu)).astype(BF16)
            par, a0 = tidx(t)
            dq = _nn(kT_s[par, hl, pl.ds(a0, KP)], ds)
            dkT_s[par, hl, pl.ds(a0, KP)] += _nt(qbd[u * UL:(u + 1) * UL], ds)
            dvT_s[par, hl, pl.ds(a0, KP)] += _nt(dos[u * UL:(u + 1) * UL].astype(BF16), pn)
            return dq

        def bwd_step(t, tn, src, dst):
            qi, q0, l0 = idx(t)
            dos = prep(t)
            e = dos * oT_s[t]
            dosn = prep(tn)
            qg = q_s[pl.ds(q0, QP), pl.ds(l0, 128)].astype(F32)
            qbd = spread(qg, lambda hp: slot_of_lane == hp).T.astype(BF16)
            parts = []
            for u in range(NU):
                dp_u(tn, dosn, dst, u)
                parts.append(ds_u(t, dos, e, qbd, src, u))
            dqt = jnp.concatenate(parts, axis=0)
            dq_s[pl.ds(q0, QP), pl.ds(l0, 128)] = (gather(dqt.T) * SCALE).astype(BF16)

        def bwd_body(i, c2):
            t = 2 * i
            bwd_step(t, t + 1, bufA, bufB)
            bwd_step(t + 1, jnp.minimum(t + 2, NT - 1), bufB, bufA)
            return c2

        with jax.named_scope("attn_bwd"):
            dos0 = prep(0)
            for u in range(NU):
                dp_u(0, dos0, bufA, u)
            lax.fori_loop(0, NT // 2, bwd_body, 0)
        return carry

    with jax.named_scope("p2_all"):
        lax.fori_loop(0, NSB, p2, 0)

    def p3(c, carry):
        r0 = pl.multiple_of(c * RC, RC)
        rows = pl.ds(r0, RC)
        dqkv_s[rows, 0:D] = dq_s[rows, :]
        a = pl.multiple_of(r0 + W - 128, 128)
        dk = dkT_s[0, :, pl.ds(r0 + W, RC)].T + dkT_s[1, :, pl.ds(a, RC + 128)].T[128 - QP:128 - QP + RC]
        dv = dvT_s[0, :, pl.ds(r0 + W, RC)].T + dvT_s[1, :, pl.ds(a, RC + 128)].T[128 - QP:128 - QP + RC]
        dqkv_s[rows, D:2 * D] = (dk * (1.0 / LOG2E)).astype(BF16)
        dqkv_s[rows, 2 * D:3 * D] = dv.astype(BF16)
        dy1 = _nt(dqkv_s[rows, :], wqkv_ref[...])
        x = x_ref[rows, :].astype(F32)
        y1, r1 = _ln(x)
        dx_ref[rows, :] = (dh_s[rows, :] + _ln_bwd(dy1, y1, r1)).astype(BF16)
        dx_copy(c).start()
        return carry

    with jax.named_scope("p3"):
        lax.fori_loop(0, S // RC, p3, 0)

    with jax.named_scope("p4_wgrad"):
        dwqkv_ref[...] = _tn(ln1_s[...], dqkv_s[...]).astype(BF16)
        dw_copies[0].start()
        dwg_ref[...] = _tn(dg_s[...], ln2_s[...]).astype(BF16)
        dw_copies[1].start()
        dwu_ref[...] = _tn(du_s[...], ln2_s[...]).astype(BF16)
        dw_copies[2].start()
        dwd_ref[...] = _tn(hh_s[...], go_ref[...]).astype(BF16)
        dw_copies[3].start()
        dwo_ref[...] = _tn(o_s[...], dh_s[...].astype(BF16)).astype(BF16)
        dw_copies[4].start()
    for i in range(NSB):
        out_copy(i).wait()
    for i in range(S // RC):
        dx_copy(i).wait()
    for cp in dw_copies:
        cp.wait()


@jax.jit
def pallas_sequential_preLN__sliding_block__glu_gated_glu__prompt_kernel(
    A_x: jax.Array,
    A_wqkv: jax.Array,
    A_wo: jax.Array,
    B_x: jax.Array,
    B_w_gate: jax.Array,
    B_w_up: jax.Array,
    B_w_down: jax.Array,
    grad_out: jax.Array,
):
    del B_x
    x = A_x.reshape(S, D)
    go = grad_out.reshape(S, D)
    sds = jax.ShapeDtypeStruct
    out_shape = (
        sds((S, D), BF16), sds((S, D), BF16),
        sds((D, 3 * D), BF16), sds((D, D), BF16),
        sds((F, D), BF16), sds((F, D), BF16), sds((F, D), BF16),
    )
    scratch = [
        pltpu.VMEM((S, D), BF16), pltpu.VMEM((D, 3 * D), BF16), pltpu.VMEM((D, D), BF16),
        pltpu.VMEM((F, D), BF16), pltpu.VMEM((F, D), BF16), pltpu.VMEM((F, D), BF16),
        pltpu.VMEM((S, D), BF16),
        pltpu.VMEM((S, D), BF16), pltpu.VMEM((S, D), BF16),
        pltpu.VMEM((D, 3 * D), BF16), pltpu.VMEM((D, D), BF16),
        pltpu.VMEM((F, D), BF16), pltpu.VMEM((F, D), BF16), pltpu.VMEM((F, D), BF16),
        pltpu.SemaphoreType.DMA((7,)), pltpu.SemaphoreType.DMA((NSB,)),
        pltpu.SemaphoreType.DMA((S // RC,)), pltpu.SemaphoreType.DMA((5,)),
        pltpu.VMEM((S, D), BF16),
        pltpu.VMEM((S, D), BF16),
        pltpu.VMEM((S + W + PADT, D), BF16),
        pltpu.VMEM((2, D, S + W), BF16),
        pltpu.VMEM((S + W + PADT, D), BF16),
        pltpu.VMEM((2, D, S + W), BF16),
        pltpu.VMEM((S, D), BF16),
        pltpu.VMEM((NT, 128, 128), F32),
        pltpu.VMEM((NT, 128, 128), F32),
        pltpu.VMEM((NT, NU, KP, 128), BF16),
        pltpu.VMEM((SB, D), F32),
        pltpu.VMEM((S, D), BF16),
        pltpu.VMEM((S, F), BF16),
        pltpu.VMEM((S, F), BF16),
        pltpu.VMEM((S, F), BF16),
        pltpu.VMEM((S, D), F32),
        pltpu.VMEM((S, D), BF16),
        pltpu.VMEM((2, D, S + W), F32),
        pltpu.VMEM((2, D, S + W), F32),
        pltpu.VMEM((S, 3 * D), BF16),
        pltpu.VMEM((NU, KP, 128), F32),
        pltpu.VMEM((NU, KP, 128), F32),
        pltpu.VMEM((NVAR, KP, 128), F32),
    ]
    outs = pl.pallas_call(
        _kernel,
        out_shape=out_shape,
        in_specs=[pl.BlockSpec(memory_space=pl.ANY)] * 7,
        out_specs=tuple(pl.BlockSpec(memory_space=pl.ANY) for _ in range(7)),
        scratch_shapes=scratch,
        compiler_params=pltpu.CompilerParams(vmem_limit_bytes=120 * 1024 * 1024),
    )(x, A_wqkv, A_wo, B_w_gate.T, B_w_up.T, B_w_down, go)
    out, dx = outs[0].reshape(1, S, D), outs[1].reshape(1, S, D)
    return (out, dx, outs[2], outs[3], outs[4].T, outs[5].T, outs[6])
```

```python
import jax
import jax.numpy as jnp
from jax import lax
import jax.experimental.pallas as pl
import jax.experimental.pallas.tpu as pltpu

S, D, F = 2048, 512, 1376
H, DH, W = 32, 16, 256
QB = 128
KW = QB + W
NG = D // 128
HG = 128 // DH
SB = 512
NSB = S // SB
NT = (SB // QB) * NG
RC = 512
DC = 256
EPS = 1e-5
NEG = -1e9
SCALE = DH ** -0.5
LOG2E = 1.4426950408889634
F32 = jnp.float32
BF16 = jnp.bfloat16


def _nn(a, b):
    return jnp.dot(a, b, preferred_element_type=F32)


def _nt(a, b):
    return lax.dot_general(a, b, (((1,), (1,)), ((), ())), preferred_element_type=F32)


def _tn(a, b):
    return lax.dot_general(a, b, (((0,), (0,)), ((), ())), preferred_element_type=F32)


def _ln(x):
    m = jnp.mean(x, axis=-1, keepdims=True)
    xc = x - m
    v = jnp.mean(xc * xc, axis=-1, keepdims=True)
    r = lax.rsqrt(v + EPS)
    return xc * r, r


def _ln_bwd(dy, y, r):
    a = jnp.mean(dy, axis=-1, keepdims=True)
    b = jnp.mean(dy * y, axis=-1, keepdims=True)
    return r * (dy - a - y * b)


def _kernel(x_hbm, wqkv_hbm, wo_hbm, wg_hbm, wu_hbm, wd_hbm, go_hbm,
            out_hbm, dx_hbm, dwqkv_hbm, dwo_hbm, dwg_hbm, dwu_hbm, dwd_hbm,
            x_ref, wqkv_ref, wo_ref, wg_ref, wu_ref, wd_ref, go_ref,
            out_ref, dx_ref, dwqkv_ref, dwo_ref, dwg_ref, dwu_ref, dwd_ref,
            in_sems, x_sems, out_sems, dx_sems, dw_sems,
            ln1_s, q_s, qT_s, k_s, kT_s, v_s, vT_s, o_s, oT_s, il_s, p_s, doT_s, ln2_s, hh_s,
            dg_s, du_s, dh_s, dq_s, dkT_s, dvT_s, dqkv_s, bufA, bufB, mb_s):
    in_pairs = [(wqkv_hbm, wqkv_ref), (wo_hbm, wo_ref), (wg_hbm, wg_ref),
                (wu_hbm, wu_ref), (wd_hbm, wd_ref), (go_hbm, go_ref)]
    in_copies = [pltpu.make_async_copy(src, dst, in_sems.at[i])
                 for i, (src, dst) in enumerate(in_pairs)]
    def x_copy(i):
        r = pl.ds(pl.multiple_of(i * RC, RC), RC)
        return pltpu.make_async_copy(x_hbm.at[r, :], x_ref.at[r, :], x_sems.at[i])

    in_copies[0].start()
    for i in range(S // RC):
        x_copy(i).start()

    def out_copy(i):
        r = pl.ds(pl.multiple_of(i * SB, SB), SB)
        return pltpu.make_async_copy(out_ref.at[r, :], out_hbm.at[r, :], out_sems.at[i])

    def dx_copy(i):
        r = pl.ds(pl.multiple_of(i * RC, RC), RC)
        return pltpu.make_async_copy(dx_ref.at[r, :], dx_hbm.at[r, :], dx_sems.at[i])

    dw_pairs = [(dwqkv_ref, dwqkv_hbm), (dwg_ref, dwg_hbm), (dwu_ref, dwu_hbm),
                (dwd_ref, dwd_hbm), (dwo_ref, dwo_hbm)]
    dw_copies = [pltpu.make_async_copy(src, dst, dw_sems.at[i])
                 for i, (src, dst) in enumerate(dw_pairs)]

    k_s[0:W, :] = jnp.zeros((W, D), BF16)
    v_s[0:W, :] = jnp.zeros((W, D), BF16)
    kT_s[:, 0:W] = jnp.zeros((D, W), BF16)
    vT_s[:, 0:W] = jnp.zeros((D, W), BF16)
    dkT_s[...] = jnp.zeros(dkT_s.shape, F32)
    dvT_s[...] = jnp.zeros(dvT_s.shape, F32)

    c_i = lax.broadcasted_iota(jnp.int32, (KW, QB), 0)
    r_i = lax.broadcasted_iota(jnp.int32, (KW, QB), 1)
    for var in range(3):
        ok = (c_i > r_i) & (c_i <= r_i + W) & (c_i >= (2 - var) * QB)
        mb_s[var] = jnp.where(ok, 0.0, NEG)

    def p1(c, carry):
        r0 = pl.multiple_of(c * RC, RC)
        x_copy(c).wait()
        x = x_ref[pl.ds(r0, RC), :].astype(F32)
        y, _ = _ln(x)
        yb = y.astype(BF16)
        ln1_s[pl.ds(r0, RC), :] = yb
        qkv = _nn(yb, wqkv_ref[...])
        q = qkv[:, 0:D]
        k = qkv[:, D:2 * D]
        v = qkv[:, 2 * D:3 * D]
        q_s[pl.ds(r0, RC), :] = (q * (SCALE * LOG2E)).astype(BF16)
        k_s[pl.ds(r0 + W, RC), :] = k.astype(BF16)
        v_s[pl.ds(r0 + W, RC), :] = v.astype(BF16)
        qT_s[:, pl.ds(r0, RC)] = (q * SCALE).T.astype(BF16)
        kT_s[:, pl.ds(r0 + W, RC)] = k.T.astype(BF16)
        vT_s[:, pl.ds(r0 + W, RC)] = v.T.astype(BF16)
        return carry

    in_copies[0].wait()
    for cp in in_copies[1:]:
        cp.start()
    with jax.named_scope("p1_qkv"):
        lax.fori_loop(0, S // RC, p1, 0)
    for cp in in_copies[1:]:
        cp.wait()

    head_of_lane = lax.broadcasted_iota(jnp.int32, (QB, 128), 1) // DH
    head_of_row = lax.broadcasted_iota(jnp.int32, (128, QB), 0) // DH

    def p2(sb, carry):
        r0 = pl.multiple_of(sb * SB, SB)

        def idx(t):
            qi = sb * (SB // QB) + t // NG
            g = t % NG
            return qi, pl.multiple_of(qi * QB, QB), pl.multiple_of(g * 128, 128)

        def qk_j(t, dst, j):
            qi, q0, l0 = idx(t)
            qg = q_s[pl.ds(q0, QB), pl.ds(l0, 128)]
            kg = k_s[pl.ds(q0, KW), pl.ds(l0, 128)]
            qm = jnp.where(head_of_lane == j, qg, jnp.zeros_like(qg))
            dst[j] = _nt(kg, qm) + mb_s[jnp.minimum(qi, 2)]

        def sm_pv_j(t, src, j):
            qi, q0, l0 = idx(t)
            s = src[j]
            m = jnp.max(s, axis=0, keepdims=True)
            p = jnp.exp2(s - m)
            il = 1.0 / jnp.sum(p, axis=0, keepdims=True)
            pn = p.astype(BF16)
            p_s[t, j] = pn
            vt = vT_s[pl.ds(pl.multiple_of(l0 + j * DH, DH), DH), pl.ds(q0, KW)]
            return _nn(vt, pn) * il, jnp.broadcast_to(il, (DH, QB))

        def fwd_step(t, tn, src, dst):
            qi, q0, l0 = idx(t)
            o_parts, il_parts = [], []
            for j in range(HG):
                qk_j(tn, dst, j)
                o, il = sm_pv_j(t, src, j)
                o_parts.append(o)
                il_parts.append(il)
            ot = jnp.concatenate(o_parts, axis=0)
            oT_s[t] = ot
            il_s[t] = jnp.concatenate(il_parts, axis=0)
            o_s[pl.ds(q0, QB), pl.ds(l0, 128)] = ot.T.astype(BF16)

        def fwd_body(i, c2):
            t = 2 * i
            fwd_step(t, t + 1, bufA, bufB)
            fwd_step(t + 1, jnp.minimum(t + 2, NT - 1), bufB, bufA)
            return c2

        with jax.named_scope("attn_fwd"):
            for j in range(HG):
                qk_j(0, bufA, j)
            lax.fori_loop(0, NT // 2, fwd_body, 0, unroll=4)

        def dense(ci, c2):
            d0 = pl.multiple_of(r0 + ci * DC, DC)
            rows = pl.ds(d0, DC)
            x = x_ref[rows, :].astype(F32)
            h = x + _nn(o_s[rows, :], wo_ref[...])
            y2, r2 = _ln(h)
            y2b = y2.astype(BF16)
            ln2_s[rows, :] = y2b
            gt = _nt(y2b, wg_ref[...])
            u = _nt(y2b, wu_ref[...])
            sg = jax.nn.sigmoid(gt)
            hh = (sg * u).astype(BF16)
            hh_s[rows, :] = hh
            out_ref[rows, :] = (h + _nn(hh, wd_ref[...])).astype(BF16)

            go = go_ref[rows, :]
            dhh = _nt(go, wd_ref[...])
            du = dhh * sg
            dg = du * u * (1.0 - sg)
            dub = du.astype(BF16)
            dgb = dg.astype(BF16)
            du_s[rows, :] = dub
            dg_s[rows, :] = dgb
            dy2 = _nn(dgb, wg_ref[...]) + _nn(dub, wu_ref[...])
            dh = go.astype(F32) + _ln_bwd(dy2, y2, r2)
            dh_s[rows, :] = dh
            doT_s[:, pl.ds(pl.multiple_of(ci * DC, DC), DC)] = _nt(wo_ref[...], dh.astype(BF16))
            return c2

        with jax.named_scope("dense"):
            lax.fori_loop(0, SB // DC, dense, 0)
        out_copy(sb).start()

        def prep(t):
            b0 = pl.multiple_of((t // NG) * QB, QB)
            l0 = pl.multiple_of((t % NG) * 128, 128)
            dos = doT_s[pl.ds(l0, 128), pl.ds(b0, QB)] * il_s[t]
            return dos

        def dp_j(t, dos, dst, j):
            qi, q0, l0 = idx(t)
            vg = v_s[pl.ds(q0, KW), pl.ds(l0, 128)]
            wj = jnp.where(head_of_row == j, dos, 0.0).astype(BF16)
            dst[j] = _nn(vg, wj)

        def ds_j(t, dos, e, src, j):
            qi, q0, l0 = idx(t)
            hl = pl.ds(pl.multiple_of(l0 + j * DH, DH), DH)
            ej = jnp.sum(e[j * DH:(j + 1) * DH], axis=0, keepdims=True)
            pn = p_s[t, j]
            ds = (pn.astype(F32) * (src[j] - ej)).astype(BF16)
            dq = _nn(kT_s[hl, pl.ds(q0, KW)], ds)
            dkT_s[hl, pl.ds(q0, KW)] += _nt(qT_s[hl, pl.ds(q0, QB)], ds)
            dvT_s[hl, pl.ds(q0, KW)] += _nt(dos[j * DH:(j + 1) * DH].astype(BF16), pn)
            return dq

        def bwd_step(t, tn, src, dst):
            qi, q0, l0 = idx(t)
            dos = prep(t)
            e = dos * oT_s[t]
            dosn = prep(tn)
            parts = []
            for j in range(HG):
                dp_j(tn, dosn, dst, j)
                parts.append(ds_j(t, dos, e, src, j))
            dqt = jnp.concatenate(parts, axis=0) * SCALE
            dq_s[pl.ds(q0, QB), pl.ds(l0, 128)] = dqt.T.astype(BF16)

        def bwd_body(i, c2):
            t = 2 * i
            bwd_step(t, t + 1, bufA, bufB)
            bwd_step(t + 1, jnp.minimum(t + 2, NT - 1), bufB, bufA)
            return c2

        with jax.named_scope("attn_bwd"):
            dos0 = prep(0)
            for j in range(HG):
                dp_j(0, dos0, bufA, j)
            lax.fori_loop(0, NT // 2, bwd_body, 0, unroll=2)
        return carry

    with jax.named_scope("p2_all"):
        lax.fori_loop(0, NSB, p2, 0)

    def p3(c, carry):
        r0 = pl.multiple_of(c * RC, RC)
        rows = pl.ds(r0, RC)
        dqkv_s[rows, 0:D] = dq_s[rows, :]
        dqkv_s[rows, D:2 * D] = dkT_s[:, pl.ds(r0 + W, RC)].T.astype(BF16)
        dqkv_s[rows, 2 * D:3 * D] = dvT_s[:, pl.ds(r0 + W, RC)].T.astype(BF16)
        dy1 = _nt(dqkv_s[rows, :], wqkv_ref[...])
        x = x_ref[rows, :].astype(F32)
        y1, r1 = _ln(x)
        dx_ref[rows, :] = (dh_s[rows, :] + _ln_bwd(dy1, y1, r1)).astype(BF16)
        dx_copy(c).start()
        return carry

    with jax.named_scope("p3"):
        lax.fori_loop(0, S // RC, p3, 0)

    with jax.named_scope("p4_wgrad"):
        dwqkv_ref[...] = _tn(ln1_s[...], dqkv_s[...]).astype(BF16)
        dw_copies[0].start()
        dwg_ref[...] = _tn(dg_s[...], ln2_s[...]).astype(BF16)
        dw_copies[1].start()
        dwu_ref[...] = _tn(du_s[...], ln2_s[...]).astype(BF16)
        dw_copies[2].start()
        dwd_ref[...] = _tn(hh_s[...], go_ref[...]).astype(BF16)
        dw_copies[3].start()
        dwo_ref[...] = _tn(o_s[...], dh_s[...].astype(BF16)).astype(BF16)
        dw_copies[4].start()
    for i in range(NSB):
        out_copy(i).wait()
    for i in range(S // RC):
        dx_copy(i).wait()
    for cp in dw_copies:
        cp.wait()


@jax.jit
def pallas_sequential_preLN__sliding_block__glu_gated_glu__prompt_kernel(
    A_x: jax.Array,
    A_wqkv: jax.Array,
    A_wo: jax.Array,
    B_x: jax.Array,
    B_w_gate: jax.Array,
    B_w_up: jax.Array,
    B_w_down: jax.Array,
    grad_out: jax.Array,
):
    del B_x
    x = A_x.reshape(S, D)
    go = grad_out.reshape(S, D)
    sds = jax.ShapeDtypeStruct
    out_shape = (
        sds((S, D), BF16), sds((S, D), BF16),
        sds((D, 3 * D), BF16), sds((D, D), BF16),
        sds((F, D), BF16), sds((F, D), BF16), sds((F, D), BF16),
    )
    scratch = [
        pltpu.VMEM((S, D), BF16), pltpu.VMEM((D, 3 * D), BF16), pltpu.VMEM((D, D), BF16),
        pltpu.VMEM((F, D), BF16), pltpu.VMEM((F, D), BF16), pltpu.VMEM((F, D), BF16),
        pltpu.VMEM((S, D), BF16),
        pltpu.VMEM((S, D), BF16), pltpu.VMEM((S, D), BF16),
        pltpu.VMEM((D, 3 * D), BF16), pltpu.VMEM((D, D), BF16),
        pltpu.VMEM((F, D), BF16), pltpu.VMEM((F, D), BF16), pltpu.VMEM((F, D), BF16),
        pltpu.SemaphoreType.DMA((6,)), pltpu.SemaphoreType.DMA((S // RC,)),
        pltpu.SemaphoreType.DMA((NSB,)),
        pltpu.SemaphoreType.DMA((S // RC,)), pltpu.SemaphoreType.DMA((5,)),
        pltpu.VMEM((S, D), BF16),
        pltpu.VMEM((S, D), BF16),
        pltpu.VMEM((D, S), BF16),
        pltpu.VMEM((S + W, D), BF16),
        pltpu.VMEM((D, S + W), BF16),
        pltpu.VMEM((S + W, D), BF16),
        pltpu.VMEM((D, S + W), BF16),
        pltpu.VMEM((S, D), BF16),
        pltpu.VMEM((NT, 128, QB), F32),
        pltpu.VMEM((NT, 128, QB), F32),
        pltpu.VMEM((NT, HG, KW, QB), BF16),
        pltpu.VMEM((D, SB), F32),
        pltpu.VMEM((S, D), BF16),
        pltpu.VMEM((S, F), BF16),
        pltpu.VMEM((S, F), BF16),
        pltpu.VMEM((S, F), BF16),
        pltpu.VMEM((S, D), F32),
        pltpu.VMEM((S, D), BF16),
        pltpu.VMEM((D, S + W), F32),
        pltpu.VMEM((D, S + W), F32),
        pltpu.VMEM((S, 3 * D), BF16),
        pltpu.VMEM((HG, KW, QB), F32),
        pltpu.VMEM((HG, KW, QB), F32),
        pltpu.VMEM((3, KW, QB), F32),
    ]
    outs = pl.pallas_call(
        _kernel,
        out_shape=out_shape,
        in_specs=[pl.BlockSpec(memory_space=pl.ANY)] * 7,
        out_specs=tuple(pl.BlockSpec(memory_space=pl.ANY) for _ in range(7)),
        scratch_shapes=scratch,
        compiler_params=pltpu.CompilerParams(vmem_limit_bytes=120 * 1024 * 1024),
    )(x, A_wqkv, A_wo, B_w_gate.T, B_w_up.T, B_w_down, go)
    out, dx = outs[0].reshape(1, S, D), outs[1].reshape(1, S, D)
    return (out, dx, outs[2], outs[3], outs[4].T, outs[5].T, outs[6])
```
